```python
import jax
import jax.numpy as jnp

def _softmax(x, axis=-1):
    return jax.nn.softmax(x, axis=axis)
def _gelu(x):
    return jax.nn.gelu(x, approximate=True)
def _silu(x):
    return jax.nn.silu(x)
def _sigmoid(x):
    return jax.nn.sigmoid(x)
def _layernorm(x, axis=-1, eps=1e-5):
    m = jnp.mean(x, axis=axis, keepdims=True)
    v = jnp.var(x, axis=axis, keepdims=True)
    return (x - m) / jnp.sqrt(v + eps)
def _scatter_add(tgt, idx, src, axis=0):
    return tgt.at[idx].add(src)
def _segment_sum(src, seg, n):
    return jax.ops.segment_sum(src, seg, n)
class _Rng:
    def __init__(self, key):
        self._k = key
    def _next(self):
        self._k, sub = jax.random.split(self._k)
        return sub
    def normal(self, shape):
        return jax.random.normal(self._next(), shape, dtype=jnp.bfloat16)
    def randint(self, lo, hi, shape):
        return jax.random.randint(self._next(), shape, lo, hi, dtype=jnp.int32)
    def uniform(self, shape, lo=0.0, hi=1.0):
        return jax.random.uniform(self._next(), shape, jnp.bfloat16, lo, hi)
    def permutation(self, n):
        return jax.random.permutation(self._next(), n)


kernel_name = 'interleave_layers__sliding_local_dilated__glu_gated_swiglu__prompt'

def setup_inputs():
    _rng = _Rng(jax.random.key(int.from_bytes(__import__("os").urandom(4), "little")))
    _w = (lambda a: (lambda t: t.astype(jnp.bfloat16) if jnp.issubdtype(t.dtype, jnp.floating) else t)(jnp.asarray(a)))
    def _A_setup():
        B, S, D = 1, 2048, 1024
        return {
            "x": _w((lambda *s: _rng.normal(s) * 0.05)(B, S, D)),
            "wqkv": _w((lambda *s: _rng.normal(s) * 0.05)(D, 3 * D)),
            "wo": _w((lambda *s: _rng.normal(s) * 0.05)(D, D)),
        }
    _A_in = _A_setup()

    def _B_setup():
        B, S, D, F = 1, 2048, 1024, 3584
        return {
            "x": _w((lambda *s: _rng.normal(s) * 0.05)(B, S, D)),
            "w1": _w((lambda *s: _rng.normal(s) * 0.05)(D, F) * (2.0 / D) ** 0.5),
            "w3": _w((lambda *s: _rng.normal(s) * 0.05)(D, F) * (2.0 / D) ** 0.5),
            "w2": _w((lambda *s: _rng.normal(s) * 0.05)(F, D) * (2.0 / F) ** 0.5),
        }
    _B_in = _B_setup()

    return {
        "A_x": _A_in["x"],
        "A_wqkv": _A_in["wqkv"],
        "A_wo": _A_in["wo"],
        "B_x": _B_in["x"],
        "B_w1": _B_in["w1"],
        "B_w3": _B_in["w3"],
        "B_w2": _B_in["w2"],
    }

def reference(A_x, A_wqkv, A_wo, B_x, B_w1, B_w3, B_w2):
    def _A_ref(x, wqkv, wo):
        B, S, D = x.shape
        H = 32; Dh = D // H
        W, dil = 8, 2
        qkv = (lambda x, *d: x.transpose(*d))((x @ wqkv).reshape(B, S, 3, H, Dh), 2, 0, 3, 1, 4)
        q, k, v = qkv[0], qkv[1], qkv[2]
        scale = Dh ** -0.5
        pos = jnp.arange(S)
        off = jnp.arange(W) * dil
        idx = pos[:, None] - off[None, :]
        mask = idx >= 0
        idx_c = jnp.where(mask, idx, 0).reshape(-1)
        kg = k[:, :, idx_c, :].reshape(B, H, S, W, Dh)
        vg = v[:, :, idx_c, :].reshape(B, H, S, W, Dh)
        logits = jnp.einsum("bhsd,bhswd->bhsw", q, kg) * scale
        logits = jnp.where(mask[None, None, :, :], logits, -1e9)
        attn = _softmax(logits, axis=-1)
        o = jnp.einsum("bhsw,bhswd->bhsd", attn, vg)
        return (lambda x, *d: x.transpose(*d))(o, 0, 2, 1, 3).reshape(B, S, D) @ wo

    def _B_ref(x, w1, w3, w2):
        gate = jnp.einsum("bsd,df->bsf", x, w1)
        up = jnp.einsum("bsd,df->bsf", x, w3)
        h = _silu(gate) * up
        out = jnp.einsum("bsf,fd->bsd", h, w2)
        return out

    x = A_x
    x = x + _A_ref(_layernorm(x, axis=-1), A_wqkv, A_wo)
    x = x + _B_ref(_layernorm(x, axis=-1), B_w1, B_w3, B_w2)
    x = x + _A_ref(_layernorm(x, axis=-1), A_wqkv, A_wo)
    x = x + _B_ref(_layernorm(x, axis=-1), B_w1, B_w3, B_w2)
    return x
```

```python
import functools
import numpy as np
import jax
import jax.numpy as jnp
from jax import lax
import jax.experimental.pallas as pl
import jax.experimental.pallas.tpu as pltpu

H, W, DIL = 32, 8, 2
HALO = 16
EPS = 1e-5
LOG2E = 1.4426950408889634
NEG = -1e9 * LOG2E


def _ln(x):
    m = jnp.mean(x, axis=-1, keepdims=True)
    c = x - m
    v = jnp.mean(c * c, axis=-1, keepdims=True)
    return c * lax.rsqrt(v + EPS)


def _dot(a, b):
    return jnp.dot(a, b, preferred_element_type=jnp.float32)


def make(TM=256, FC=512, RA=32, LNR=32, DC=256, QC=512, sig=0, flags=None, skip='', nloop=None, prof=False, prio=0, PU=1, AD=0):
    names = ['x0', 'x1', 'xr', 'wq', 'wk', 'wv', 'wo', 'w1', 'w3', 'w2']

    def kernel(x_hbm, wqkv_hbm, wo_hbm, w1_hbm, w3_hbm, w2_hbm, out_hbm,
               xv, ov, wqkv, wo, w1, w3, w2, tbuf, xres, xn1, xn2, qs, ks, vs, os_, hs, sems, osems):
        S, D = xres.shape
        F = w1.shape[-1]
        NT = D // 128
        NB = S // TM
        Dh = D // H

        NU = 2 * NB

        def cp(name):
            i = names.index(name)
            if name in ('wq', 'wk', 'wv'):
                j = ('wq', 'wk', 'wv').index(name)
                src, dst = wqkv_hbm.at[:, pl.ds(j * D, D)], wqkv.at[j]
            elif name in ('x0', 'x1', 'xr'):
                r = {'x0': pl.ds(0, TM), 'x1': pl.ds(TM, TM), 'xr': pl.ds(2 * TM, S - 2 * TM)}[name]
                src, dst = x_hbm.at[r], xv.at[r]
            else:
                src, dst = {'wo': (wo_hbm, wo), 'w1': (w1_hbm, w1), 'w3': (w3_hbm, w3), 'w2': (w2_hbm, w2)}[name]
            return pltpu.make_async_copy(src, dst, sems.at[i])

        def start(*ns):
            for n in ns:
                cp(n).start(priority=prio)

        def wait(*ns):
            if prof:
                with jax.named_scope('S_' + ns[0]):
                    for n in ns:
                        cp(n).wait()
                return
            for n in ns:
                cp(n).wait()

        def out_cp(b):
            r = pl.multiple_of(b * TM, TM) if not isinstance(b, int) else b * TM
            return pltpu.make_async_copy(ov.at[pl.ds(r, TM)], out_hbm.at[pl.ds(r, TM)], osems.at[b])

        def gather_rows(tb):
            return jnp.concatenate([tb[pl.ds(d, H, stride=Dh), :] for d in range(Dh)], axis=0)

        def permute_qkv(i):
            def body(r, c):
                for k in range(PU):
                    tb = tbuf.at[k]
                    rows = pl.ds(pl.multiple_of((r * PU + k) * 256, 256), 256)
                    tb[...] = pltpu.bitcast(wqkv[i, rows, :], jnp.uint32).T
                    wqkv[i, rows, :] = pltpu.bitcast(gather_rows(tb).T, jnp.bfloat16)
                return c
            lax.fori_loop(0, D // 256 // PU, body, 0)

        def permute_wo():
            def body(j, c):
                tb = tbuf.at[0]
                cols = pl.ds(pl.multiple_of(j * 128, 128), 128)
                tb[...] = pltpu.bitcast(wo[:, cols].astype(jnp.float32), jnp.uint32)
                wo[:, cols] = pltpu.bitcast(gather_rows(tb), jnp.float32).astype(jnp.bfloat16)
                return c
            lax.fori_loop(0, NT, body, 0)

        def rows_of(u):
            return pl.multiple_of(lax.rem(u + NB, NB) * TM, TM)

        def x_in(u, r0, n, cols=slice(None)):
            rows = pl.ds(rows_of(u) + r0, n)
            return jnp.where(u < NB, xv[rows, cols].astype(jnp.float32), xres[rows, cols])

        def ln1(u, r0):
            xn1[pl.ds(r0, LNR), :] = _ln(x_in(u, r0, LNR)).astype(jnp.bfloat16)

        def ln2(u, r0):
            xn2[pl.ds(r0, LNR), :] = _ln(xres[pl.ds(rows_of(u) + r0, LNR), :]).astype(jnp.bfloat16)

        def proj(u, i, c0):
            y = _dot(xn1[...], wqkv[i, :, c0:c0 + QC])
            for jj in range(QC // 128):
                j = c0 // 128 + jj
                yj = y[:, jj * 128:(jj + 1) * 128]
                if i == 0:
                    qs[j] = yj * (Dh ** -0.5 * LOG2E)
                else:
                    buf = ks if i == 1 else vs
                    head = jnp.broadcast_to(yj[0:1, :], (HALO, 128))
                    buf[j, pl.ds(0, HALO), :] = jnp.where(lax.rem(u, NB) == 0, head, buf[j, pl.ds(TM, HALO), :])
                    buf[j, pl.ds(HALO, TM), :] = yj

        def attn(u, r0):
            static = isinstance(r0, int)
            lg = []
            for w in range(W):
                acc = None
                for j in range(NT):
                    p = qs[j, pl.ds(r0, RA), :] * ks[j, pl.ds(r0 + (HALO - DIL * w), RA), :]
                    acc = p if acc is None else acc + p
                acc = acc + pltpu.roll(acc, 64, 1)
                acc = acc + pltpu.roll(acc, 32, 1)
                if w > 0 and (not static or r0 < DIL * w):
                    pos = rows_of(u) + r0 + lax.broadcasted_iota(jnp.int32, (RA, 128), 0)
                    acc = jnp.where(pos >= DIL * w, acc, NEG)
                lg.append(acc)
            m = functools.reduce(jnp.maximum, lg)
            e = [jnp.exp2(v - m) for v in lg]
            inv = 1.0 / functools.reduce(lambda a_, b_: a_ + b_, e)
            p = [v * inv for v in e]
            for j in range(NT):
                acc = None
                for w in range(W):
                    v = p[w] * vs[j, pl.ds(r0 + (HALO - DIL * w), RA), :]
                    acc = v if acc is None else acc + v
                os_[pl.ds(r0, RA), j * 128:(j + 1) * 128] = acc.astype(jnp.bfloat16)

        def oproj(u, c0):
            cols = slice(c0, c0 + QC)
            xres[pl.ds(rows_of(u), TM), cols] = x_in(u, 0, TM, cols) + _dot(os_[...], wo[:, cols])

        def gate_up(c0):
            cols = pl.ds(c0, FC)
            a = xn2[...]
            g = _dot(a, w1[:, cols])
            u = _dot(a, w3[:, cols])
            hs[:, cols] = (g * jax.nn.sigmoid(g) * u).astype(jnp.bfloat16)

        def down(u, c0):
            cols = slice(c0, c0 + DC)
            rows = pl.ds(rows_of(u), TM)
            y = xres[rows, cols] + _dot(hs[...], w2[:, cols])
            xres[rows, cols] = y
            ov[rows, cols] = y.astype(ov.dtype)

        def row_loop(fn, u, n):
            def body(r, c):
                fn(u, pl.multiple_of(r * n, n))
                return c
            lax.fori_loop(0, TM // n, body, 0)

        def spread(mxu_tasks, vpu_tasks):
            n, m = len(mxu_tasks), len(vpu_tasks)
            for i, task in enumerate(mxu_tasks):
                task()
                for v in vpu_tasks[i * m // n:(i + 1) * m // n]:
                    v()

        P = functools.partial

        start('x0', 'wq')
        xres[pl.ds(S - TM, TM), :] = jnp.zeros((TM, D), jnp.float32)
        for buf in (ks, vs):
            buf[:, pl.ds(TM, HALO), :] = jnp.zeros((NT, HALO, 128), jnp.float32)
        wait('x0')
        start('wk')

        def ln1_first(u, r0):
            xn1[pl.ds(r0, LNR), :] = _ln(xv[pl.ds(r0, LNR), :].astype(jnp.float32)).astype(jnp.bfloat16)
        row_loop(ln1_first, 0, LNR)
        wait('wq')
        start('wv')
        permute_qkv(0)
        wait('wk')
        start('wo', 'x1')
        permute_qkv(1)
        wait('wv')
        start('w1', 'w3')
        permute_qkv(2)

        def period(t, carry):
            @pl.when(t < NU)
            def _():
                spread([P(proj, t, i, c0) for i in range(3) for c0 in range(0, D, QC)],
                       [P(ln2, t - 1, r0) for r0 in range(0, TM, LNR)])

            @pl.when(t == NU)
            def _():
                row_loop(ln2, t - 1, LNR)

            @pl.when(t == 0)
            def _():
                row_loop(attn, t, RA)
                wait('wo', 'x1')
                start('w2', 'xr')
                permute_wo()

            @pl.when(t == 1)
            def _():
                wait('w1', 'w3')

            @pl.when(t > 0)
            def _():
                def wait_w2():
                    pl.when(t == 1)(lambda: wait('w2', 'xr'))
                gu = [P(gate_up, c0) for c0 in range(0, F, FC)]
                dn = [P(down, t - 1, c0) for c0 in range(0, D, DC)]
                at = [P(attn, t, r0) for r0 in range(0, TM, RA)]
                if AD:
                    k = len(at) * AD // 8
                    spread(gu, at[:len(at) - k])
                    wait_w2()
                    spread(dn, at[len(at) - k:])
                else:
                    spread(gu, at)
                    wait_w2()
                    spread(dn, [])

            @pl.when(t > NB)
            def _():
                out_cp(t - 1 - NB).start()

            @pl.when(t < NU)
            def _():
                for r0 in range(0, TM, LNR):
                    ln1(t + 1, r0)
                for c0 in range(0, D, QC):
                    oproj(t, c0)
            return carry

        lax.fori_loop(0, NU + 1, period, 0)
        if prof:
            with jax.named_scope('S_end'):
                out_cp(NB - 1).wait()
        for b in range(NB - 1 if prof else NB):
            out_cp(b).wait()

    @jax.jit
    def run(A_x, A_wqkv, A_wo, B_x, B_w1, B_w3, B_w2):
        B, S, D = A_x.shape
        F = B_w1.shape[1]
        NT = D // 128
        NB = S // TM
        bf, f32 = jnp.bfloat16, jnp.float32
        anyspec = pl.BlockSpec(memory_space=pl.ANY)
        out = pl.pallas_call(
            kernel,
            in_specs=[anyspec] * 6,
            out_specs=anyspec,
            out_shape=jax.ShapeDtypeStruct((S, D), A_x.dtype),
            scratch_shapes=[
                pltpu.VMEM((S, D), bf), pltpu.VMEM((S, D), bf),
                pltpu.VMEM((3, D, D), bf), pltpu.VMEM((D, D), bf),
                pltpu.VMEM((D, F), bf), pltpu.VMEM((D, F), bf), pltpu.VMEM((F, D), bf),
                pltpu.VMEM((PU, D, 128), jnp.uint32),
                pltpu.VMEM((S, D), f32),
                pltpu.VMEM((TM, D), bf), pltpu.VMEM((TM, D), bf),
                pltpu.VMEM((NT, TM, 128), f32),
                pltpu.VMEM((NT, TM + HALO, 128), f32), pltpu.VMEM((NT, TM + HALO, 128), f32),
                pltpu.VMEM((TM, D), bf), pltpu.VMEM((TM, F), bf),
                pltpu.SemaphoreType.DMA((len(names),)), pltpu.SemaphoreType.DMA((NB,)),
            ],
            compiler_params=pltpu.CompilerParams(
                vmem_limit_bytes=100 * 1024 * 1024, flags=flags),
        )(A_x.reshape(S, D), A_wqkv, A_wo, B_w1, B_w3, B_w2)
        return out.reshape(B, S, D)
    return run


_run = make(AD=3)


@jax.jit
def pallas_interleave_layers__sliding_local_dilated__glu_gated_swiglu__prompt_kernel(
    A_x, A_wqkv, A_wo, B_x, B_w1, B_w3, B_w2
):
    return _run(A_x, A_wqkv, A_wo, B_x, B_w1, B_w3, B_w2)
```

```python
import functools
import numpy as np
import jax
import jax.numpy as jnp
from jax import lax
import jax.experimental.pallas as pl
import jax.experimental.pallas.tpu as pltpu

H, W, DIL = 32, 8, 2
HALO = 16
EPS = 1e-5
FL = {'E': 'XLA_TPU_EVENLY_DISTRIBUTE_CRITICAL_NODES', 'R': 'XLA_TPU_RESCHEDULE_DMA_DONES', 'F': 'XLA_TPU_ENABLE_LLO_SMALL_LOOP_FLATTENING'}
LOG2E = 1.4426950408889634
NEG = -1e9 * LOG2E


def _ln(x):
    m = jnp.mean(x, axis=-1, keepdims=True)
    c = x - m
    v = jnp.mean(c * c, axis=-1, keepdims=True)
    return c * lax.rsqrt(v + EPS)


def _dot(a, b):
    return jnp.dot(a, b, preferred_element_type=jnp.float32)


def make(TM=256, FC=512, RA=32, LNR=32, DC=256, QC=512, sig=0, flags='E', skip='', nloop=None, prof=False, prio=0, PU=2, TK=0, AD=0, alias='1', OC=512, sh=2, bar='', PW=4, order=2):
    names = ['x0', 'x1', 'xr', 'wo', 'w1', 'w3', 'w2']

    def kernel(x_hbm, wqkv_hbm, wo_hbm, w1_hbm, w3_hbm, w2_hbm, out_hbm,
               xv, ov, wqkv, wo, w1, w3, w2, tbuf, xres, act, qs, ks, vs, hs, sems, osems, qsems, *tok):
        S, D = xres.shape
        F = w1.shape[-1]
        NT = D // 128
        NB = S // TM
        Dh = D // H

        NU = 2 * NB

        def cp(name):
            i = names.index(name)
            if name in ('x0', 'x1', 'xr'):
                r = {'x0': pl.ds(0, TM), 'x1': pl.ds(TM, TM), 'xr': pl.ds(2 * TM, S - 2 * TM)}[name]
                src, dst = x_hbm.at[r], xv.at[r]
            else:
                src, dst = {'wo': (wo_hbm, wo), 'w1': (w1_hbm, w1), 'w3': (w3_hbm, w3), 'w2': (w2_hbm, w2)}[name]
            return pltpu.make_async_copy(src, dst, sems.at[i])

        def start(*ns):
            for n in ns:
                cp(n).start(priority=prio)

        def wait(*ns):
            if prof:
                with jax.named_scope('S_' + ns[0]):
                    for n in ns:
                        cp(n).wait()
                return
            for n in ns:
                cp(n).wait()

        NP = 3 * (D // 256)

        def piece(n):
            i, r = n // (D // 256), n % (D // 256)
            if not isinstance(n, int):
                return i, pl.multiple_of(r * 256, 256), pl.multiple_of(i * D, D)
            return i, r * 256, i * D

        def qkv_cp(n):
            i, r0, c0 = piece(n)
            return pltpu.make_async_copy(wqkv_hbm.at[pl.ds(r0, 256), pl.ds(c0, D)],
                                         wqkv.at[i, pl.ds(r0, 256), :], qsems.at[n])

        def out_cp(b):
            r = pl.multiple_of(b * TM, TM) if not isinstance(b, int) else b * TM
            return pltpu.make_async_copy(ov.at[pl.ds(r, TM)], out_hbm.at[pl.ds(r, TM)], osems.at[b])

        def scatter_rows(tb, v, n):
            for g in range(v.shape[0] // n):
                tb[pl.ds(g * (n + 1), n), :] = v[g * n:(g + 1) * n]

        def permute_qkv(n, tb):
            i, r0, _ = piece(n)
            scatter_rows(tb, pltpu.bitcast(wqkv[i, pl.ds(r0, 256), :], jnp.uint32).T, Dh)
            rows = [tb[pl.ds(d, H, stride=Dh + 1), :] for d in range(Dh)]
            wqkv[i, pl.ds(r0, 256), :] = pltpu.bitcast(jnp.concatenate(rows, axis=0).T, jnp.bfloat16)

        def permute_wo(j, tb):
            cols = pl.ds(pl.multiple_of(j * 128, 128), 128)
            scatter_rows(tb, pltpu.bitcast(wo[:, cols], jnp.uint32), Dh)
            out = []
            for e in range(Dh // 2):
                a = tb[pl.ds(e, H // 2, stride=Dh + 1), :]
                b = tb[pl.ds(Dh // 2 + e, H // 2, stride=Dh + 1), :]
                out.append((a & 0xFFFF) | (b << 16))
                out.append((a >> 16) | (b & jnp.uint32(0xFFFF0000)))
            wo[:, cols] = pltpu.bitcast(jnp.concatenate(out, axis=0), jnp.bfloat16)

        def rows_of(u):
            return pl.multiple_of(lax.rem(u + NB, NB) * TM, TM)

        def x_in(u, r0, n, cols=slice(None)):
            rows = pl.ds(rows_of(u) + r0, n)
            return jnp.where(u < NB, xv[rows, cols].astype(jnp.float32), xres[rows, cols])

        xn2 = act.at[0]

        def mark(name):
            if prof:
                with jax.named_scope('S_' + name):
                    tbuf[0, pl.ds(0, 8), :] = jnp.zeros((8, 128), jnp.uint32)

        def fence(u, tag):
            if tag in bar:
                pl.when(u < -1)(lambda: wait('x0'))

        def lhs(slot, u):
            if str(slot) not in alias:
                return act[slot]
            return jnp.concatenate([act[slot + (u >> 8), pl.ds(0, 16), :], act[slot, pl.ds(16, TM - 16), :]], axis=0)

        def ln1(u, r0):
            act[1, pl.ds(r0, LNR), :] = _ln(x_in(u, r0, LNR)).astype(jnp.bfloat16)

        def ln2(u, r0):
            y = _ln(xres[pl.ds(rows_of(u) + r0, LNR), :]).astype(jnp.bfloat16)
            xn2[pl.ds(r0, LNR), :] = y
            if isinstance(r0, int) and r0 == 0:
                for tk in tok:
                    tk[pl.ds(0, 16), :] = y[:16]

        def proj(u, i, c0):
            y = _dot(lhs(1, u), wqkv[i, :, c0:c0 + QC])
            fence(u, 'p')
            for jj in range(QC // 128):
                j = c0 // 128 + jj
                yj = y[:, jj * 128:(jj + 1) * 128]
                if i == 0:
                    qs[j] = yj * (Dh ** -0.5 * LOG2E)
                else:
                    buf = ks if i == 1 else vs
                    head = jnp.broadcast_to(yj[0:1, :], (HALO, 128))
                    buf[j, pl.ds(0, HALO), :] = jnp.where(lax.rem(u, NB) == 0, head, buf[j, pl.ds(TM, HALO), :])
                    buf[j, pl.ds(HALO, TM), :] = yj

        def attn(u, r0):
            static = isinstance(r0, int)

            def windows(buf, j):
                out = [None] * W
                for sft in range(0, 8, DIL):
                    base = buf[j, pl.ds(r0 + (HALO - 8 - sft), RA + 8), :]
                    out[sft // DIL] = base[8:]
                    out[(sft + 8) // DIL] = base[:RA]
                return out

            lg = [None] * W
            for j in range(NT):
                qj = qs[j, pl.ds(r0, RA), :]
                kw = windows(ks, j)
                for w in range(W):
                    p = qj * kw[w]
                    lg[w] = p if j == 0 else lg[w] + p
            for w in range(W):
                acc = lg[w]
                acc = acc + pltpu.roll(acc, 64, 1)
                acc = acc + pltpu.roll(acc, 32, 1)
                if w > 0 and (not static or r0 < DIL * w):
                    pos = rows_of(u) + r0 + lax.broadcasted_iota(jnp.int32, (RA, 128), 0)
                    acc = jnp.where(pos >= DIL * w, acc, NEG)
                lg[w] = acc
            m = functools.reduce(jnp.maximum, lg)
            e = [jnp.exp2(v - m) for v in lg]
            inv = 1.0 / functools.reduce(lambda a_, b_: a_ + b_, e)
            p = [v * inv for v in e]
            for j in range(NT):
                vw = windows(vs, j)
                acc = p[0] * vw[0]
                for w in range(1, W):
                    acc = acc + p[w] * vw[w]
                if TK and static:
                    tok[r0 // RA][pl.ds(16, RA), j * 128:(j + 1) * 128] = acc.astype(jnp.bfloat16)
                else:
                    act[2, pl.ds(r0, RA), j * 128:(j + 1) * 128] = acc.astype(jnp.bfloat16)

        def oproj(u, c0):
            cols = slice(c0, c0 + OC)
            a = jnp.concatenate([tk[pl.ds(16, RA), :] for tk in tok], axis=0) if TK else lhs(2, u)
            y = _dot(a, wo[:, cols])
            fence(u, 'o')
            xres[pl.ds(rows_of(u), TM), cols] = x_in(u, 0, TM, cols) + y

        def gate_up(u, c0, after=None):
            cols = pl.ds(c0, FC)
            a = lhs(0, u)
            if after is not None:
                head = tok[after][pl.ds(pl.multiple_of((u >> 8) * 16, 16), 16), :]
                a = jnp.concatenate([head, act[0, pl.ds(16, TM - 16), :]], axis=0)
            g = _dot(a, w1[:, cols])
            up = _dot(a, w3[:, cols])
            fence(u, 'g')
            hs[:, cols] = (g * jax.nn.sigmoid(g) * up).astype(jnp.bfloat16)

        def down(u, c0):
            cols = slice(c0, c0 + DC)
            rows = pl.ds(rows_of(u), TM)
            y = _dot(hs[...], w2[:, cols])
            fence(u, 'd')
            y = xres[rows, cols] + y
            xres[rows, cols] = y
            ov[rows, cols] = y.astype(ov.dtype)

        def row_loop(fn, u, n):
            def body(r, c):
                fn(u, pl.multiple_of(r * n, n))
                return c
            lax.fori_loop(0, TM // n, body, 0)

        def spread(mxu_tasks, vpu_tasks):
            n, m = len(mxu_tasks) - sh, len(vpu_tasks)
            for i, task in enumerate(mxu_tasks):
                task()
                for v in vpu_tasks[i * m // n:(i + 1) * m // n]:
                    v()

        P = functools.partial

        for n in range(PW):
            qkv_cp(n).start()
        start('x0')
        xres[pl.ds(S - TM, TM), :] = jnp.zeros((TM, D), jnp.float32)
        for buf in (ks, vs):
            buf[:, pl.ds(TM, HALO), :] = jnp.zeros((NT, HALO, 128), jnp.float32)

        def ln1_first(u, r0):
            rows = pl.ds(u * TM + r0, LNR)
            act[1, pl.ds(r0, LNR), :] = _ln(xv[rows, :].astype(jnp.float32)).astype(jnp.bfloat16)

        NI = NP // PU
        LPI = -(-(TM // LNR) // NI)

        def prep(it, c):
            for k in range(PU):
                qkv_cp(it * PU + k).wait()
            for k in range(PU):
                n = it * PU + k + PW
                pl.when(n < NP)(lambda: qkv_cp(n).start())
            pl.when(it == NI - 2)(lambda: start('wo', 'x1'))
            pl.when(it == NI - 1)(lambda: start('w1', 'w3'))
            pl.when(it == 0)(lambda: wait('x0'))
            for k in range(PU):
                permute_qkv(it * PU + k, tbuf.at[k])
            for k in range(LPI):
                r = jnp.minimum(it * LPI + k, TM // LNR - 1)
                ln1_first(0, pl.multiple_of(r * LNR, LNR))
            return c
        lax.fori_loop(0, NI, prep, 0)
        mark('prep')

        def period(t, carry):
            @pl.when(t < NU)
            def _():
                spread([P(proj, t, i, c0) for i in range(3) for c0 in range(0, D, QC)],
                       [P(ln2, t - 1, r0) for r0 in range(0, TM, LNR)])

            @pl.when(t == NU)
            def _():
                row_loop(ln2, t - 1, LNR)
                for tk in tok:
                    tk[pl.ds(0, 16), :] = act[0, pl.ds(0, 16), :]

            @pl.when(t == 0)
            def _():
                wait('wo', 'x1')
                start('w2', 'xr')

                def body(r, c):
                    for k in range(TM // NT // RA):
                        attn(t, pl.multiple_of(r * (TM // NT) + k * RA, RA))
                    for k in range(TM // NT // LNR):
                        ln1_first(1, pl.multiple_of(r * (TM // NT) + k * LNR, LNR))
                    permute_wo(r, tbuf.at[0])
                    return c
                lax.fori_loop(0, NT, body, 0)
                mark('att')

                def body2(c, cc):
                    cols = pl.ds(pl.multiple_of(c * 256, 256), 256)
                    xres[pl.ds(0, TM), cols] = xv[pl.ds(0, TM), cols].astype(jnp.float32) + _dot(act[2], wo[:, cols])
                    return cc
                lax.fori_loop(0, D // 256, body2, 0)
                mark('op')

            @pl.when(t == 1)
            def _():
                wait('w1', 'w3')

            pl.when((t >= 2) & (t < 4))(lambda: mark('A'))
            at = [P(attn, t, r0) for r0 in range(0, TM, RA)]

            @pl.when(t > 0)
            def _():
                if TK:
                    nc = F // FC
                    done = 0
                    for c in range(nc):
                        hi = min(len(at), (c * len(at) + TK - 1) // TK)
                        for k in range(done, hi):
                            at[k]()
                        gate_up(t, c * FC, hi - 1 if hi > done else None)
                        done = hi
                    for k in range(done, len(at)):
                        at[k]()
                else:
                    spread([P(gate_up, t, c0) for c0 in range(0, F, FC)], at)

            pl.when((t >= 2) & (t < 4))(lambda: mark('B'))
            @pl.when(t == 1)
            def _():
                wait('w2', 'xr')

            @pl.when(t > 0)
            def _():
                dn = [P(down, t - 1, c0) for c0 in range(0, D, DC)]
                op = [P(oproj, t, c0) for c0 in range(0, D, OC)]
                ln = [P(ln1, t + 1, r0) for r0 in range(0, TM, LNR)]
                if order == 0:
                    spread(ln + dn + op, [])
                elif order == 1:
                    spread(ln + op + dn, [])
                else:
                    spread(op + dn, ln)

            pl.when(((t >= 1) & (t < 4)) | (t > 14))(lambda: mark('C'))
            @pl.when(t > NB)
            def _():
                out_cp(t - 1 - NB).start()
            return carry

        lax.fori_loop(0, NU + 1, period, 0)
        if prof:
            with jax.named_scope('S_end'):
                out_cp(NB - 1).wait()
        for b in range(NB - 1 if prof else NB):
            out_cp(b).wait()

    @jax.jit
    def run(A_x, A_wqkv, A_wo, B_x, B_w1, B_w3, B_w2):
        B, S, D = A_x.shape
        F = B_w1.shape[1]
        NT = D // 128
        NB = S // TM
        bf, f32 = jnp.bfloat16, jnp.float32
        anyspec = pl.BlockSpec(memory_space=pl.ANY)
        out = pl.pallas_call(
            kernel,
            in_specs=[anyspec] * 6,
            out_specs=anyspec,
            out_shape=jax.ShapeDtypeStruct((S, D), A_x.dtype),
            scratch_shapes=[
                pltpu.VMEM((S, D), bf), pltpu.VMEM((S, D), bf),
                pltpu.VMEM((3, D, D), bf), pltpu.VMEM((D, D), bf),
                pltpu.VMEM((D, F), bf), pltpu.VMEM((D, F), bf), pltpu.VMEM((F, D), bf),
                pltpu.VMEM((PU, D + H, 128), jnp.uint32),
                pltpu.VMEM((S, D), f32),
                pltpu.VMEM((3, TM, D), bf),
                pltpu.VMEM((NT, TM, 128), f32),
                pltpu.VMEM((NT, TM + HALO, 128), f32), pltpu.VMEM((NT, TM + HALO, 128), f32),
                pltpu.VMEM((TM, F), bf),
                pltpu.SemaphoreType.DMA((len(names),)), pltpu.SemaphoreType.DMA((NB,)),
                pltpu.SemaphoreType.DMA((3 * (D // 256),)),
            ] + [pltpu.VMEM((16 + RA, D), bf) for _ in range(TM // RA if TK else 0)
            ],
            compiler_params=pltpu.CompilerParams(
                vmem_limit_bytes=100 * 1024 * 1024, flags={FL[c]: True for c in flags}),
        )(A_x.reshape(S, D), A_wqkv, A_wo, B_w1, B_w3, B_w2)
        return out.reshape(B, S, D)
    return run


_run = make(alias='')


@jax.jit
def pallas_interleave_layers__sliding_local_dilated__glu_gated_swiglu__prompt_kernel(
    A_x, A_wqkv, A_wo, B_x, B_w1, B_w3, B_w2
):
    return _run(A_x, A_wqkv, A_wo, B_x, B_w1, B_w3, B_w2)
```

```python
import functools
import numpy as np
import jax
import jax.numpy as jnp
from jax import lax
import jax.experimental.pallas as pl
import jax.experimental.pallas.tpu as pltpu

H, W, DIL = 32, 8, 2
HALO = 16
EPS = 1e-5
FL = {'E': 'XLA_TPU_EVENLY_DISTRIBUTE_CRITICAL_NODES', 'R': 'XLA_TPU_RESCHEDULE_DMA_DONES', 'F': 'XLA_TPU_ENABLE_LLO_SMALL_LOOP_FLATTENING'}
LOG2E = 1.4426950408889634
NEG = -1e9 * LOG2E


def _ln(x):
    m = jnp.mean(x, axis=-1, keepdims=True)
    c = x - m
    v = jnp.mean(c * c, axis=-1, keepdims=True)
    return c * lax.rsqrt(v + EPS)


def _dot(a, b):
    return jnp.dot(a, b, preferred_element_type=jnp.float32)


def make(TM=256, FC=512, RA=32, LNR=32, DC=256, QC=512, sig=0, flags='E', skip='', nloop=None, prof=False, prio=0, PU=2, TK=0, AD=0, alias='1', OC=512, sh=2, bar='', PW=4, order=2):
    names = ['x0', 'x1', 'xr', 'wo', 'w1', 'w3', 'w2']

    def kernel(x_hbm, wqkv_hbm, wo_hbm, w1_hbm, w3_hbm, w2_hbm, out_hbm,
               xv, ov, wqkv, wo, w1, w3, w2, tbuf, xres, xn1, xn2, ao, qkv, hs, sems, osems, qsems):
        S, D = xres.shape
        F = w1.shape[-1]
        NT = D // 128
        NB = S // TM
        Dh = D // H
        QSCALE = Dh ** -0.5 * LOG2E

        NU = 2 * NB

        def cp(name):
            i = names.index(name)
            if name in ('x0', 'x1', 'xr'):
                r = {'x0': pl.ds(0, TM), 'x1': pl.ds(TM, TM), 'xr': pl.ds(2 * TM, S - 2 * TM)}[name]
                src, dst = x_hbm.at[r], xv.at[r]
            else:
                src, dst = {'wo': (wo_hbm, wo), 'w1': (w1_hbm, w1), 'w3': (w3_hbm, w3), 'w2': (w2_hbm, w2)}[name]
            return pltpu.make_async_copy(src, dst, sems.at[i])

        def start(*ns):
            for n in ns:
                cp(n).start(priority=prio)

        def wait(*ns):
            if prof:
                with jax.named_scope('S_' + ns[0]):
                    for n in ns:
                        cp(n).wait()
                return
            for n in ns:
                cp(n).wait()

        NP = 3 * (D // 256)

        def piece(n):
            i, r = n // (D // 256), n % (D // 256)
            if not isinstance(n, int):
                return i, pl.multiple_of(r * 256, 256), pl.multiple_of(i * D, D)
            return i, r * 256, i * D

        def qkv_cp(n):
            i, r0, c0 = piece(n)
            return pltpu.make_async_copy(wqkv_hbm.at[pl.ds(r0, 256), pl.ds(c0, D)],
                                         wqkv.at[i, pl.ds(r0, 256), :], qsems.at[n])

        def out_cp(b):
            r = pl.multiple_of(b * TM, TM) if not isinstance(b, int) else b * TM
            return pltpu.make_async_copy(ov.at[pl.ds(r, TM)], out_hbm.at[pl.ds(r, TM)], osems.at[b])

        def scatter_rows(tb, v, n):
            for g in range(v.shape[0] // n):
                tb[pl.ds(g * (n + 1), n), :] = v[g * n:(g + 1) * n]

        def permute_qkv(n, tb):
            i, r0, _ = piece(n)
            scatter_rows(tb, pltpu.bitcast(wqkv[i, pl.ds(r0, 256), :], jnp.uint32).T, Dh)
            rows = [tb[pl.ds(d, H, stride=Dh + 1), :] for d in range(Dh)]
            wqkv[i, pl.ds(r0, 256), :] = pltpu.bitcast(jnp.concatenate(rows, axis=0).T, jnp.bfloat16)

        def permute_wo(j, tb):
            cols = pl.ds(pl.multiple_of(j * 128, 128), 128)
            scatter_rows(tb, pltpu.bitcast(wo[:, cols], jnp.uint32), Dh)
            out = []
            for e in range(Dh // 2):
                a = tb[pl.ds(e, H // 2, stride=Dh + 1), :]
                b = tb[pl.ds(Dh // 2 + e, H // 2, stride=Dh + 1), :]
                out.append((a & 0xFFFF) | (b << 16))
                out.append((a >> 16) | (b & jnp.uint32(0xFFFF0000)))
            wo[:, cols] = pltpu.bitcast(jnp.concatenate(out, axis=0), jnp.bfloat16)

        def rows_of(u):
            if isinstance(u, int):
                return (u % NB) * TM
            return pl.multiple_of(lax.rem(u, NB) * TM, TM)

        def x_in(u, r0, n, cols=slice(None)):
            rows = pl.ds(rows_of(u) + r0, n)
            return jnp.where(u < NB, xv[rows, cols].astype(jnp.float32), xres[rows, cols])

        def mark(name):
            if prof:
                with jax.named_scope('S_' + name):
                    tbuf[0, pl.ds(0, 8), :] = jnp.zeros((8, 128), jnp.uint32)

        def ln1(u, r0):
            xn1[pl.ds(r0, LNR), :] = _ln(x_in(u, r0, LNR)).astype(jnp.bfloat16)

        def ln1_first(u, r0):
            rows = pl.ds(u * TM + r0, LNR)
            xn1[pl.ds(r0, LNR), :] = _ln(xv[rows, :].astype(jnp.float32)).astype(jnp.bfloat16)

        def ln2(u, r0):
            xn2[pl.ds(r0, LNR), :] = _ln(xres[pl.ds(rows_of(u) + r0, LNR), :]).astype(jnp.bfloat16)

        def proj(u, i, c, n):
            first = isinstance(u, int)
            c0 = c * n if isinstance(c, int) else pl.multiple_of(c * n, n)
            y = _dot(xn1[...], wqkv[i, :, pl.ds(c0, n)])
            if isinstance(i, int):
                y = y * QSCALE if i == 0 else y
            else:
                y = y * jnp.where(i == 0, QSCALE, 1.0)
            for jj in range(n // 128):
                j = i * NT + c * (n // 128) + jj
                yj = y[:, jj * 128:(jj + 1) * 128]
                if first or i > 0:
                    head = jnp.broadcast_to(yj[0:1, :], (HALO, 128))
                    if not first:
                        head = jnp.where(lax.rem(u, NB) == 0, head, qkv[j, pl.ds(TM, HALO), :])
                    qkv[j, pl.ds(0, HALO), :] = head
                qkv[j, pl.ds(HALO, TM), :] = yj

        def attn(u, r0):
            static = isinstance(r0, int)

            def windows(j):
                out = [None] * W
                for sft in range(0, 8, DIL):
                    base = qkv[j, pl.ds(r0 + (HALO - 8 - sft), RA + 8), :]
                    out[sft // DIL] = base[8:]
                    out[(sft + 8) // DIL] = base[:RA]
                return out

            lg = [None] * W
            for j in range(NT):
                qj = qkv[j, pl.ds(r0 + HALO, RA), :]
                kw = windows(NT + j)
                for w in range(W):
                    p = qj * kw[w]
                    lg[w] = p if j == 0 else lg[w] + p
            for w in range(W):
                acc = lg[w]
                acc = acc + pltpu.roll(acc, 64, 1)
                acc = acc + pltpu.roll(acc, 32, 1)
                if w > 0 and (not static or r0 < DIL * w):
                    pos = rows_of(u) + r0 + lax.broadcasted_iota(jnp.int32, (RA, 128), 0)
                    acc = jnp.where(pos >= DIL * w, acc, NEG)
                lg[w] = acc
            m = functools.reduce(jnp.maximum, lg)
            e = [jnp.exp2(v - m) for v in lg]
            inv = 1.0 / functools.reduce(lambda a_, b_: a_ + b_, e)
            p = [v * inv for v in e]
            for j in range(NT):
                vw = windows(2 * NT + j)
                acc = p[0] * vw[0]
                for w in range(1, W):
                    acc = acc + p[w] * vw[w]
                ao[pl.ds(r0, RA), j * 128:(j + 1) * 128] = acc.astype(jnp.bfloat16)

        def oproj(u, c0, n):
            cols = pl.ds(c0, n)
            xres[pl.ds(rows_of(u), TM), cols] = x_in(u, 0, TM, cols) + _dot(ao[...], wo[:, cols])

        def gate_up(c0):
            cols = pl.ds(c0, FC)
            a = xn2[...]
            g = _dot(a, w1[:, cols])
            up = _dot(a, w3[:, cols])
            hs[:, cols] = (g * jax.nn.sigmoid(g) * up).astype(jnp.bfloat16)

        def down(u, c0):
            cols = pl.ds(c0, DC)
            rows = pl.ds(rows_of(u), TM)
            y = xres[rows, cols] + _dot(hs[...], w2[:, cols])
            xres[rows, cols] = y
            ov[rows, cols] = y.astype(ov.dtype)

        def loop(n, fn):
            def body(i, c):
                fn(i)
                return c
            lax.fori_loop(0, n, body, 0)

        def spread(mxu_tasks, vpu_tasks):
            n, m = len(mxu_tasks), len(vpu_tasks)
            for i, task in enumerate(mxu_tasks):
                task()
                for v in vpu_tasks[i * m // n:(i + 1) * m // n]:
                    v()

        P = functools.partial
        NQ = D // 256

        for n in range(PW):
            qkv_cp(n).start()
        start('x0')

        def next_piece(n):
            qkv_cp(n).wait()
            pl.when(n + PW < NP)(lambda: qkv_cp(n + PW).start())
            pl.when(n + PW == NP)(lambda: start('wo', 'x1'))
            pl.when(n == NP - 1)(lambda: start('w1', 'w3'))

        def prep_q(it):
            for k in range(PU):
                next_piece(it * PU + k)
            pl.when(it == 0)(lambda: wait('x0'))
            for k in range(PU):
                permute_qkv(it * PU + k, tbuf.at[k])
            per = TM // LNR // (NQ // PU)
            for k in range(per):
                ln1_first(0, pl.multiple_of((it * per + k) * LNR, LNR))
        loop(NQ // PU, prep_q)
        mark('q')

        def proj_qk(it):
            next_piece(NQ + it)
            proj(0, it // NQ, lax.rem(it, NQ), 256)
            permute_qkv(NQ + it, tbuf.at[0])
        loop(2 * NQ, proj_qk)
        mark('k')
        wait('wo', 'x1')
        start('w2', 'xr')

        def proj_v(it):
            proj(0, 2, it, 256)
            for k in range(2):
                permute_wo(2 * it + k, tbuf.at[k])
        loop(NQ, proj_v)
        mark('v')

        def attn_first(it):
            attn(0, pl.multiple_of(it * RA, RA))
            for k in range(RA // LNR):
                ln1_first(1, pl.multiple_of(it * RA + k * LNR, LNR))
        loop(TM // RA, attn_first)
        mark('att')

        def period(t, carry):
            @pl.when(t < NU)
            def _():
                spread([P(oproj, t - 1, c0, OC) for c0 in range(0, D, OC)], [])
                spread([P(proj, t, i, c, QC) for i in range(3) for c in range(D // QC)],
                       [P(ln2, t - 1, r0) for r0 in range(0, TM, LNR)])

            @pl.when(t == NU)
            def _():
                loop(D // 256, lambda c: oproj(t - 1, pl.multiple_of(c * 256, 256), 256))
                spread([P(ln2, t - 1, r0) for r0 in range(0, TM, LNR)], [])

            pl.when(t == 1)(lambda: wait('w1', 'w3'))
            pl.when(t < 4)(lambda: mark('A'))
            spread([P(gate_up, c0) for c0 in range(0, F, FC)],
                   [P(attn, t, r0) for r0 in range(0, TM, RA)])
            pl.when(t < 4)(lambda: mark('B'))
            pl.when(t == 1)(lambda: wait('w2', 'xr'))
            spread([P(down, t - 1, c0) for c0 in range(0, D, DC)],
                   [P(ln1, t + 1, r0) for r0 in range(0, TM, LNR)])
            pl.when((t < 4) | (t > 14))(lambda: mark('C'))
            pl.when(t > NB)(lambda: out_cp(t - 1 - NB).start())
            return carry

        lax.fori_loop(1, NU + 1, period, 0)
        if prof:
            with jax.named_scope('S_end'):
                out_cp(NB - 1).wait()
        for b in range(NB - 1 if prof else NB):
            out_cp(b).wait()

    @jax.jit
    def run(A_x, A_wqkv, A_wo, B_x, B_w1, B_w3, B_w2):
        B, S, D = A_x.shape
        F = B_w1.shape[1]
        NT = D // 128
        NB = S // TM
        bf, f32 = jnp.bfloat16, jnp.float32
        anyspec = pl.BlockSpec(memory_space=pl.ANY)
        out = pl.pallas_call(
            kernel,
            in_specs=[anyspec] * 6,
            out_specs=anyspec,
            out_shape=jax.ShapeDtypeStruct((S, D), A_x.dtype),
            scratch_shapes=[
                pltpu.VMEM((S, D), bf), pltpu.VMEM((S, D), bf),
                pltpu.VMEM((3, D, D), bf), pltpu.VMEM((D, D), bf),
                pltpu.VMEM((D, F), bf), pltpu.VMEM((D, F), bf), pltpu.VMEM((F, D), bf),
                pltpu.VMEM((2, D + H, 128), jnp.uint32),
                pltpu.VMEM((S, D), f32),
                pltpu.VMEM((TM, D), bf), pltpu.VMEM((TM, D), bf), pltpu.VMEM((TM, D), bf),
                pltpu.VMEM((3 * NT, TM + HALO, 128), f32),
                pltpu.VMEM((TM, F), bf),
                pltpu.SemaphoreType.DMA((len(names),)), pltpu.SemaphoreType.DMA((NB,)),
                pltpu.SemaphoreType.DMA((3 * (D // 256),)),
            ],
            compiler_params=pltpu.CompilerParams(
                vmem_limit_bytes=100 * 1024 * 1024, flags={FL[c]: True for c in flags}),
        )(A_x.reshape(S, D), A_wqkv, A_wo, B_w1, B_w3, B_w2)
        return out.reshape(B, S, D)
    return run


_run = make()


@jax.jit
def pallas_interleave_layers__sliding_local_dilated__glu_gated_swiglu__prompt_kernel(
    A_x, A_wqkv, A_wo, B_x, B_w1, B_w3, B_w2
):
    return _run(A_x, A_wqkv, A_wo, B_x, B_w1, B_w3, B_w2)
```

```python
import functools
import numpy as np
import jax
import jax.numpy as jnp
from jax import lax
import jax.experimental.pallas as pl
import jax.experimental.pallas.tpu as pltpu

H, W, DIL = 32, 8, 2
HALO = 16
EPS = 1e-5
FL = {'E': 'XLA_TPU_EVENLY_DISTRIBUTE_CRITICAL_NODES', 'R': 'XLA_TPU_RESCHEDULE_DMA_DONES', 'F': 'XLA_TPU_ENABLE_LLO_SMALL_LOOP_FLATTENING'}
LOG2E = 1.4426950408889634
NEG = -1e9 * LOG2E


def _ln(x):
    m = jnp.mean(x, axis=-1, keepdims=True)
    c = x - m
    v = jnp.mean(c * c, axis=-1, keepdims=True)
    return c * lax.rsqrt(v + EPS)


def _dot(a, b):
    return jnp.dot(a, b, preferred_element_type=jnp.float32)


def make(TM=256, FC=512, RA=32, LNR=32, DC=256, QC=512, sig=1, flags='E', skip='', nloop=None, prof=False, prio=0, PU=2, RM=16, AD=0, alias='1', OC=512, sh=2, bar='', PW=4, order=1):
    names = ['x0', 'x1', 'xr', 'wo', 'w1', 'w3', 'w2']

    def kernel(x_hbm, wqkv_hbm, wo_hbm, w1_hbm, w3_hbm, w2_hbm, out_hbm,
               xv, ov, wqkv, wo, w1, w3, w2, tbuf, xres, xn1, xn2, ao, qkv, hs, sems, osems, qsems):
        S, D = xres.shape
        F = w1.shape[-1]
        NT = D // 128
        NB = S // TM
        Dh = D // H
        QSCALE = Dh ** -0.5 * LOG2E

        NU = 2 * NB

        def cp(name):
            i = names.index(name)
            if name in ('x0', 'x1', 'xr'):
                r = {'x0': pl.ds(0, TM), 'x1': pl.ds(TM, TM), 'xr': pl.ds(2 * TM, S - 2 * TM)}[name]
                src, dst = x_hbm.at[r], xv.at[r]
            else:
                src, dst = {'wo': (wo_hbm, wo), 'w1': (w1_hbm, w1), 'w3': (w3_hbm, w3), 'w2': (w2_hbm, w2)}[name]
            return pltpu.make_async_copy(src, dst, sems.at[i])

        def start(*ns):
            for n in ns:
                cp(n).start(priority=prio)

        def wait(*ns):
            if prof:
                with jax.named_scope('S_' + ns[0]):
                    for n in ns:
                        cp(n).wait()
                return
            for n in ns:
                cp(n).wait()

        NP = 3 * (D // 256)

        def piece(n):
            i, r = n // (D // 256), n % (D // 256)
            if not isinstance(n, int):
                return i, pl.multiple_of(r * 256, 256), pl.multiple_of(i * D, D)
            return i, r * 256, i * D

        def qkv_cp(n):
            i, r0, c0 = piece(n)
            return pltpu.make_async_copy(wqkv_hbm.at[pl.ds(r0, 256), pl.ds(c0, D)],
                                         wqkv.at[i, pl.ds(r0, 256), :], qsems.at[n])

        def out_cp(b):
            r = pl.multiple_of(b * TM, TM) if not isinstance(b, int) else b * TM
            return pltpu.make_async_copy(ov.at[pl.ds(r, TM)], out_hbm.at[pl.ds(r, TM)], osems.at[b])

        def scatter_rows(tb, v, n):
            for g in range(v.shape[0] // n):
                tb[pl.ds(g * (n + 1), n), :] = v[g * n:(g + 1) * n]

        def permute_qkv(n, tb):
            i, r0, _ = piece(n)
            scatter_rows(tb, pltpu.bitcast(wqkv[i, pl.ds(r0, 256), :], jnp.uint32).T, Dh)
            rows = [tb[pl.ds(d, H, stride=Dh + 1), :] for d in range(Dh)]
            wqkv[i, pl.ds(r0, 256), :] = pltpu.bitcast(jnp.concatenate(rows, axis=0).T, jnp.bfloat16)

        def permute_wo(j, tb):
            cols = pl.ds(pl.multiple_of(j * 128, 128), 128)
            scatter_rows(tb, pltpu.bitcast(wo[:, cols], jnp.uint32), Dh)
            out = []
            for e in range(Dh // 2):
                a = tb[pl.ds(e, H // 2, stride=Dh + 1), :]
                b = tb[pl.ds(Dh // 2 + e, H // 2, stride=Dh + 1), :]
                out.append((a & 0xFFFF) | (b << 16))
                out.append((a >> 16) | (b & jnp.uint32(0xFFFF0000)))
            wo[:, cols] = pltpu.bitcast(jnp.concatenate(out, axis=0), jnp.bfloat16)

        def rows_of(u):
            if isinstance(u, int):
                return (u % NB) * TM
            return pl.multiple_of(lax.rem(u, NB) * TM, TM)

        def x_in(u, r0, n, cols=slice(None)):
            rows = pl.ds(rows_of(u) + r0, n)
            return jnp.where(u < NB, xv[rows, cols].astype(jnp.float32), xres[rows, cols])

        def mark(name):
            if prof:
                with jax.named_scope('S_' + name):
                    tbuf[0, pl.ds(0, 8), :] = jnp.zeros((8, 128), jnp.uint32)

        def ln1(u, r0):
            xn1[pl.ds(r0, LNR), :] = _ln(x_in(u, r0, LNR)).astype(jnp.bfloat16)

        def ln1_first(u, r0):
            rows = pl.ds(u * TM + r0, LNR)
            xn1[pl.ds(r0, LNR), :] = _ln(xv[rows, :].astype(jnp.float32)).astype(jnp.bfloat16)

        def ln2(u, r0):
            xn2[pl.ds(r0, LNR), :] = _ln(xres[pl.ds(rows_of(u) + r0, LNR), :]).astype(jnp.bfloat16)

        def proj(u, i, c, n):
            first = isinstance(u, int)
            c0 = c * n if isinstance(c, int) else pl.multiple_of(c * n, n)
            y = _dot(xn1[...], wqkv[i, :, pl.ds(c0, n)])
            if isinstance(i, int):
                y = y * QSCALE if i == 0 else y
            else:
                y = y * jnp.where(i == 0, QSCALE, 1.0)
            for jj in range(n // 128):
                j = i * NT + c * (n // 128) + jj
                yj = y[:, jj * 128:(jj + 1) * 128]
                if first or i > 0:
                    head = jnp.broadcast_to(yj[0:1, :], (HALO, 128))
                    if not first:
                        head = jnp.where(lax.rem(u, NB) == 0, head, qkv[j, pl.ds(TM, HALO), :])
                    qkv[j, pl.ds(0, HALO), :] = head
                qkv[j, pl.ds(HALO, TM), :] = yj

        def attn(u, r0, RA=RA):
            static = isinstance(r0, int)

            def windows(j):
                out = [None] * W
                for sft in range(0, 8, DIL):
                    base = qkv[j, pl.ds(r0 + (HALO - 8 - sft), RA + 8), :]
                    out[sft // DIL] = base[8:]
                    out[(sft + 8) // DIL] = base[:RA]
                return out

            lg = [None] * W
            for j in range(NT):
                qj = qkv[j, pl.ds(r0 + HALO, RA), :]
                kw = windows(NT + j)
                for w in range(W):
                    p = qj * kw[w]
                    lg[w] = p if j == 0 else lg[w] + p
            for w in range(W):
                acc = lg[w]
                acc = acc + pltpu.roll(acc, 64, 1)
                acc = acc + pltpu.roll(acc, 32, 1)
                if w > 0 and (not static or r0 < DIL * w):
                    pos = rows_of(u) + r0 + lax.broadcasted_iota(jnp.int32, (RA, 128), 0)
                    acc = jnp.where(pos >= DIL * w, acc, NEG)
                lg[w] = acc
            m = functools.reduce(jnp.maximum, lg)
            e = [jnp.exp2(v - m) for v in lg]
            inv = 1.0 / functools.reduce(lambda a_, b_: a_ + b_, e)
            p = [v * inv for v in e]
            for j in range(NT):
                vw = windows(2 * NT + j)
                acc = p[0] * vw[0]
                for w in range(1, W):
                    acc = acc + p[w] * vw[w]
                ao[pl.ds(r0, RA), j * 128:(j + 1) * 128] = acc.astype(jnp.bfloat16)

        def oproj(u, c0, n):
            cols = pl.ds(c0, n)
            xres[pl.ds(rows_of(u), TM), cols] = x_in(u, 0, TM, cols) + _dot(ao[...], wo[:, cols])

        def gate_up(c0):
            cols = pl.ds(c0, FC)
            a = xn2[...]
            g = _dot(a, w1[:, cols])
            up = _dot(a, w3[:, cols])
            if sig:
                hg = 0.5 * g
                hs[:, cols] = (hg * (jnp.tanh(hg) + 1.0) * up).astype(jnp.bfloat16)
            else:
                hs[:, cols] = (g * jax.nn.sigmoid(g) * up).astype(jnp.bfloat16)

        def down(u, c0):
            cols = pl.ds(c0, DC)
            rows = pl.ds(rows_of(u), TM)
            y = xres[rows, cols] + _dot(hs[...], w2[:, cols])
            xres[rows, cols] = y
            ov[rows, cols] = y.astype(ov.dtype)

        def loop(n, fn):
            def body(i, c):
                fn(i)
                return c
            lax.fori_loop(0, n, body, 0)

        def spread(mxu_tasks, vpu_tasks):
            n, m = len(mxu_tasks), len(vpu_tasks)
            for i, task in enumerate(mxu_tasks):
                task()
                for v in vpu_tasks[i * m // n:(i + 1) * m // n]:
                    v()

        P = functools.partial
        NQ = D // 256

        for n in range(PW):
            qkv_cp(n).start()
        start('x0')

        def next_piece(n):
            qkv_cp(n).wait()
            pl.when(n + PW < NP)(lambda: qkv_cp(n + PW).start())
            pl.when(n + PW == NP)(lambda: start('wo', 'x1'))
            pl.when(n == NP - 1)(lambda: start('w1', 'w3'))

        def prep_q(it):
            for k in range(PU):
                next_piece(it * PU + k)
            pl.when(it == 0)(lambda: wait('x0'))
            for k in range(PU):
                permute_qkv(it * PU + k, tbuf.at[k])
            per = TM // LNR // (NQ // PU)
            for k in range(per):
                ln1_first(0, pl.multiple_of((it * per + k) * LNR, LNR))
        loop(NQ // PU, prep_q)
        mark('q')

        def proj_qk(it):
            next_piece(NQ + it)
            proj(0, it // NQ, lax.rem(it, NQ), 256)
            permute_qkv(NQ + it, tbuf.at[0])
        loop(2 * NQ, proj_qk)
        mark('k')
        wait('wo', 'x1')
        start('w2', 'xr')

        def proj_v(it):
            proj(0, 2, it, 256)
            for k in range(2):
                permute_wo(2 * it + k, tbuf.at[k])
        loop(NQ, proj_v)
        mark('v')

        def attn_first(it):
            attn(0, pl.multiple_of(it * RA, RA))
            for k in range(RA // LNR):
                ln1_first(1, pl.multiple_of(it * RA + k * LNR, LNR))
        loop(TM // RA, attn_first)
        mark('att')

        def period(t, carry):
            @pl.when(t < NU)
            def _():
                spread([P(oproj, t - 1, c0, OC) for c0 in range(0, D, OC)], [])
                spread([P(proj, t, i, c, QC) for i in range(3) for c in range(D // QC)],
                       [P(ln2, t - 1, r0) for r0 in range(0, TM, LNR)])

            @pl.when(t == NU)
            def _():
                loop(D // 256, lambda c: oproj(t - 1, pl.multiple_of(c * 256, 256), 256))
                spread([P(ln2, t - 1, r0) for r0 in range(0, TM, LNR)], [])

            pl.when(t == 1)(lambda: wait('w1', 'w3'))
            pl.when(t < 4)(lambda: mark('A'))
            at = [P(attn, t, r0, RM) for r0 in range(0, TM, RM)]
            k = len(at) - len(at) * AD // 8
            l1 = [P(ln1, t + 1, r0) for r0 in range(0, TM, LNR)]
            spread([P(gate_up, c0) for c0 in range(0, F, FC)], (l1 if order == 3 else []) + at[:k] + (l1 if order == 1 else []))
            pl.when(t < 4)(lambda: mark('B'))
            pl.when(t == 1)(lambda: wait('w2', 'xr'))
            spread([P(down, t - 1, c0) for c0 in range(0, D, DC)], at[k:] + (l1 if order == 2 else []))
            pl.when((t < 4) | (t > 14))(lambda: mark('C'))
            pl.when(t > NB)(lambda: out_cp(t - 1 - NB).start())
            return carry

        lax.fori_loop(1, NU + 1, period, 0)
        if prof:
            with jax.named_scope('S_end'):
                out_cp(NB - 1).wait()
        for b in range(NB - 1 if prof else NB):
            out_cp(b).wait()

    @jax.jit
    def run(A_x, A_wqkv, A_wo, B_x, B_w1, B_w3, B_w2):
        B, S, D = A_x.shape
        F = B_w1.shape[1]
        NT = D // 128
        NB = S // TM
        bf, f32 = jnp.bfloat16, jnp.float32
        anyspec = pl.BlockSpec(memory_space=pl.ANY)
        out = pl.pallas_call(
            kernel,
            in_specs=[anyspec] * 6,
            out_specs=anyspec,
            out_shape=jax.ShapeDtypeStruct((S, D), A_x.dtype),
            scratch_shapes=[
                pltpu.VMEM((S, D), bf), pltpu.VMEM((S, D), bf),
                pltpu.VMEM((3, D, D), bf), pltpu.VMEM((D, D), bf),
                pltpu.VMEM((D, F), bf), pltpu.VMEM((D, F), bf), pltpu.VMEM((F, D), bf),
                pltpu.VMEM((2, D + H, 128), jnp.uint32),
                pltpu.VMEM((S, D), f32),
                pltpu.VMEM((TM, D), bf), pltpu.VMEM((TM, D), bf), pltpu.VMEM((TM, D), bf),
                pltpu.VMEM((3 * NT, TM + HALO, 128), f32),
                pltpu.VMEM((TM, F), bf),
                pltpu.SemaphoreType.DMA((len(names),)), pltpu.SemaphoreType.DMA((NB,)),
                pltpu.SemaphoreType.DMA((3 * (D // 256),)),
            ],
            compiler_params=pltpu.CompilerParams(
                vmem_limit_bytes=100 * 1024 * 1024, flags={FL[c]: True for c in flags}),
        )(A_x.reshape(S, D), A_wqkv, A_wo, B_w1, B_w3, B_w2)
        return out.reshape(B, S, D)
    return run


_run = make()


@jax.jit
def pallas_interleave_layers__sliding_local_dilated__glu_gated_swiglu__prompt_kernel(
    A_x, A_wqkv, A_wo, B_x, B_w1, B_w3, B_w2
):
    return _run(A_x, A_wqkv, A_wo, B_x, B_w1, B_w3, B_w2)
```

```python
import functools

import jax
import jax.numpy as jnp
from jax import lax
import jax.experimental.pallas as pl
import jax.experimental.pallas.tpu as pltpu

H, W, DIL = 32, 8, 2
EPS = 1e-5
LOG2E = 1.4426950408889634
NEG = -1e9 * LOG2E
HALO = 16

TM = 256
FC = 512
DC = 256
QC = 512
RM = 16
RA = 32
LNR = 32
PR = 256
PW = 4
PU = 2

_COPIES = ('x0', 'x1', 'xr', 'wo', 'w1', 'w3', 'w2')


def _ln(x):
    m = jnp.mean(x, axis=-1, keepdims=True)
    c = x - m
    v = jnp.mean(c * c, axis=-1, keepdims=True)
    return c * lax.rsqrt(v + EPS)


def _dot(a, b):
    return jnp.dot(a, b, preferred_element_type=jnp.float32)


def _aligned(i, n):
    return i * n if isinstance(i, int) else pl.multiple_of(i * n, n)


def _loop(n, fn):
    def body(i, carry):
        fn(i)
        return carry
    lax.fori_loop(0, n, body, 0)


def _spread(mxu_tasks, vpu_tasks):
    n, m = len(mxu_tasks), len(vpu_tasks)
    for i, task in enumerate(mxu_tasks):
        task()
        for v in vpu_tasks[i * m // n:(i + 1) * m // n]:
            v()


def _kernel(x_hbm, wqkv_hbm, wo_hbm, w1_hbm, w3_hbm, w2_hbm, out_hbm,
            xv, ov, wqkv, wo, w1, w3, w2, tbuf, xres, xn1, xn2, ao, qkv, hs,
            sems, osems, qsems):
    S, D = xres.shape
    F = w1.shape[-1]
    NT = D // 128
    NB = S // TM
    NU = 2 * NB
    NQ = D // PR
    NP = 3 * NQ
    Dh = D // H
    QSCALE = Dh ** -0.5 * LOG2E
    P = functools.partial

    def copy(name):
        if name in ('x0', 'x1', 'xr'):
            r = {'x0': pl.ds(0, TM), 'x1': pl.ds(TM, 2 * TM), 'xr': pl.ds(3 * TM, S - 3 * TM)}[name]
            src, dst = x_hbm.at[r], xv.at[r]
        else:
            src, dst = {'wo': (wo_hbm, wo), 'w1': (w1_hbm, w1),
                        'w3': (w3_hbm, w3), 'w2': (w2_hbm, w2)}[name]
        return pltpu.make_async_copy(src, dst, sems.at[_COPIES.index(name)])

    def start(*names):
        for n in names:
            copy(n).start()

    def wait(*names):
        for n in names:
            copy(n).wait()

    def piece(n):
        return n // NQ, pl.ds(_aligned(n % NQ, PR), PR)

    def qkv_copy(n):
        i, rows = piece(n)
        return pltpu.make_async_copy(
            wqkv_hbm.at[rows, pl.ds(_aligned(i, D), D)], wqkv.at[i, rows, :], qsems.at[n])

    def out_copy(b):
        rows = pl.ds(_aligned(b, TM), TM)
        return pltpu.make_async_copy(ov.at[rows], out_hbm.at[rows], osems.at[b])

    def scatter_rows(tb, v):
        for g in range(v.shape[0] // Dh):
            tb[pl.ds(g * (Dh + 1), Dh), :] = v[g * Dh:(g + 1) * Dh]

    def permute_qkv(n, tb):
        i, rows = piece(n)
        scatter_rows(tb, pltpu.bitcast(wqkv[i, rows, :], jnp.uint32).T)
        t = jnp.concatenate([tb[pl.ds(d, H, stride=Dh + 1), :] for d in range(Dh)], axis=0)
        wqkv[i, rows, :] = pltpu.bitcast(t.T, jnp.bfloat16)

    def permute_wo(j, tb):
        cols = pl.ds(_aligned(j, 128), 128)
        scatter_rows(tb, pltpu.bitcast(wo[:, cols], jnp.uint32))
        out = []
        for e in range(Dh // 2):
            a = tb[pl.ds(e, H // 2, stride=Dh + 1), :]
            b = tb[pl.ds(Dh // 2 + e, H // 2, stride=Dh + 1), :]
            out.append((a & 0xFFFF) | (b << 16))
            out.append((a >> 16) | ((b >> 16) << 16))
        wo[:, cols] = pltpu.bitcast(jnp.concatenate(out, axis=0), jnp.bfloat16)

    def rows_of(u):
        return _aligned(u % NB, TM)

    def x_in(u, r0, n, cols=slice(None)):
        rows = pl.ds(rows_of(u) + r0, n)
        return jnp.where(u < NB, xv[rows, cols].astype(jnp.float32), xres[rows, cols])

    def ln1(u, r0):
        xn1[pl.ds(r0, LNR), :] = _ln(x_in(u, r0, LNR)).astype(jnp.bfloat16)

    def ln1_first(u, r0):
        x = xv[pl.ds(u * TM + r0, LNR), :].astype(jnp.float32)
        xn1[pl.ds(r0, LNR), :] = _ln(x).astype(jnp.bfloat16)

    def ln2(u, r0):
        xn2[pl.ds(r0, LNR), :] = _ln(xres[pl.ds(rows_of(u) + r0, LNR), :]).astype(jnp.bfloat16)

    def proj(u, i, c, n):
        first = isinstance(u, int) and u == 0
        y = _dot(xn1[...], wqkv[i, :, pl.ds(_aligned(c, n), n)])
        if isinstance(i, int):
            y = y * QSCALE if i == 0 else y
        else:
            y = y * jnp.where(i == 0, QSCALE, 1.0)
        for jj in range(n // 128):
            j = i * NT + c * (n // 128) + jj
            yj = y[:, jj * 128:(jj + 1) * 128]
            if first or i > 0:
                head = jnp.broadcast_to(yj[0:1, :], (HALO, 128))
                if not first:
                    head = jnp.where(u % NB == 0, head, qkv[j, pl.ds(TM, HALO), :])
                qkv[j, pl.ds(0, HALO), :] = head
            qkv[j, pl.ds(HALO, TM), :] = yj

    def attn(u, r0, n):
        def taps(j):
            out = [None] * W
            for shift in range(0, 8, DIL):
                base = qkv[j, pl.ds(r0 + (HALO - 8 - shift), n + 8), :]
                out[shift // DIL] = base[8:]
                out[(shift + 8) // DIL] = base[:n]
            return out

        lg = [None] * W
        for j in range(NT):
            q = qkv[j, pl.ds(r0 + HALO, n), :]
            for w, k in enumerate(taps(NT + j)):
                lg[w] = q * k if j == 0 else lg[w] + q * k
        for w in range(W):
            a = lg[w]
            a = a + pltpu.roll(a, 2 * H, 1)
            a = a + pltpu.roll(a, H, 1)
            if w > 0 and (not isinstance(r0, int) or r0 < DIL * w):
                pos = rows_of(u) + r0 + lax.broadcasted_iota(jnp.int32, (n, 128), 0)
                a = jnp.where(pos >= DIL * w, a, NEG)
            lg[w] = a
        m = functools.reduce(jnp.maximum, lg)
        e = [jnp.exp2(a - m) for a in lg]
        inv = 1.0 / functools.reduce(jnp.add, e)
        p = [a * inv for a in e]
        for j in range(NT):
            o = functools.reduce(jnp.add, [pw * v for pw, v in zip(p, taps(2 * NT + j))])
            ao[pl.ds(r0, n), j * 128:(j + 1) * 128] = o.astype(jnp.bfloat16)

    def oproj(u, c, n):
        cols = pl.ds(_aligned(c, n), n)
        xres[pl.ds(rows_of(u), TM), cols] = x_in(u, 0, TM, cols) + _dot(ao[...], wo[:, cols])

    def gate_up(c):
        cols = pl.ds(c * FC, FC)
        a = xn2[...]
        hg = 0.5 * _dot(a, w1[:, cols])
        up = _dot(a, w3[:, cols])
        hs[:, cols] = (hg * (jnp.tanh(hg) + 1.0) * up).astype(jnp.bfloat16)

    def down(u, c):
        rows, cols = pl.ds(rows_of(u), TM), pl.ds(c * DC, DC)
        y = xres[rows, cols] + _dot(hs[...], w2[:, cols])
        xres[rows, cols] = y
        ov[rows, cols] = y.astype(ov.dtype)

    for n in range(PW):
        qkv_copy(n).start()
    start('x0')

    def next_pieces(n0):
        for k in range(PU):
            n = n0 + k
            qkv_copy(n).wait()
            pl.when(n + PW < NP)(lambda n=n: qkv_copy(n + PW).start())
            pl.when(n + PW == NP)(lambda: start('wo', 'x1', 'w1', 'w3'))

    def prepare_q(it):
        next_pieces(it * PU)
        pl.when(it == 0)(lambda: wait('x0'))
        for k in range(PU):
            permute_qkv(it * PU + k, tbuf.at[k])
        per = TM // LNR // (NQ // PU)
        for k in range(per):
            ln1_first(0, _aligned(it * per + k, LNR))
    _loop(NQ // PU, prepare_q)

    def project_qk(it):
        next_pieces(NQ + it * PU)
        proj(0, it // (NQ // PU), it % (NQ // PU), PU * PR)
        for k in range(PU):
            permute_qkv(NQ + it * PU + k, tbuf.at[k])
    _loop(2 * NQ // PU, project_qk)
    wait('wo', 'x1')

    def project_v(it):
        proj(0, 2, it, D // 2)
        for k in range(NT // 2):
            permute_wo(it * (NT // 2) + k, tbuf.at[k])
    _loop(2, project_v)

    def attend_first(it):
        attn(0, _aligned(it, RA), RA)
        for k in range(RA // LNR):
            ln1_first(1, _aligned(it * (RA // LNR) + k, LNR))
    _loop(TM // RA, attend_first)

    def period(t, carry):
        norm2 = [P(ln2, t - 1, r0) for r0 in range(0, TM, LNR)]

        @pl.when(t < NU)
        def _():
            for c in range(D // QC):
                oproj(t - 1, c, QC)
            _spread([P(proj, t, i, c, QC) for i in range(3) for c in range(D // QC)], norm2)

        @pl.when(t == NU)
        def _():
            _loop(D // 256, lambda c: oproj(t - 1, c, 256))
            for task in norm2:
                task()

        @pl.when(t == 1)
        def _():
            wait('w1', 'w3')
            start('w2', 'xr')

        _spread([P(gate_up, c) for c in range(F // FC)],
                [P(ln1, t + 1, r0) for r0 in range(0, TM, LNR)]
                + [P(attn, t, r0, RM) for r0 in range(0, TM, RM)])
        pl.when(t == 1)(lambda: wait('w2', 'xr'))
        for c in range(D // DC):
            down(t - 1, c)
        pl.when(t > NB)(lambda: out_copy(t - 1 - NB).start())
        return carry

    lax.fori_loop(1, NU + 1, period, 0)
    for b in range(NB):
        out_copy(b).wait()


@jax.jit
def pallas_interleave_layers__sliding_local_dilated__glu_gated_swiglu__prompt_kernel(
    A_x: jax.Array,
    A_wqkv: jax.Array,
    A_wo: jax.Array,
    B_x: jax.Array,
    B_w1: jax.Array,
    B_w3: jax.Array,
    B_w2: jax.Array,
):
    del B_x
    B, S, D = A_x.shape
    F = B_w1.shape[1]
    assert B == 1 and D == 32 * H and S % TM == 0 and S > 3 * TM and F % FC == 0
    bf16, f32 = jnp.bfloat16, jnp.float32
    hbm = pl.BlockSpec(memory_space=pl.ANY)
    out = pl.pallas_call(
        _kernel,
        in_specs=[hbm] * 6,
        out_specs=hbm,
        out_shape=jax.ShapeDtypeStruct((S, D), A_x.dtype),
        scratch_shapes=[
            pltpu.VMEM((S, D), bf16),
            pltpu.VMEM((S, D), bf16),
            pltpu.VMEM((3, D, D), bf16),
            pltpu.VMEM((D, D), bf16),
            pltpu.VMEM((D, F), bf16),
            pltpu.VMEM((D, F), bf16),
            pltpu.VMEM((F, D), bf16),
            pltpu.VMEM((D // 256, D + H, 128), jnp.uint32),
            pltpu.VMEM((S, D), f32),
            pltpu.VMEM((TM, D), bf16),
            pltpu.VMEM((TM, D), bf16),
            pltpu.VMEM((TM, D), bf16),
            pltpu.VMEM((3 * D // 128, HALO + TM, 128), f32),
            pltpu.VMEM((TM, F), bf16),
            pltpu.SemaphoreType.DMA((len(_COPIES),)),
            pltpu.SemaphoreType.DMA((S // TM,)),
            pltpu.SemaphoreType.DMA((3 * D // PR,)),
        ],
        compiler_params=pltpu.CompilerParams(
            vmem_limit_bytes=100 * 1024 * 1024,
            flags={"XLA_TPU_EVENLY_DISTRIBUTE_CRITICAL_NODES": True},
        ),
    )(A_x.reshape(S, D), A_wqkv, A_wo, B_w1, B_w3, B_w2)
    return out.reshape(B, S, D)
```

```python
import functools

import jax
import jax.numpy as jnp
from jax import lax
import jax.experimental.pallas as pl
import jax.experimental.pallas.tpu as pltpu

H, W, DIL = 32, 8, 2
EPS = 1e-5
LOG2E = 1.4426950408889634
NEG = -1e9 * LOG2E
HALO = 16

TM = 256
FC = 512
DC = 256
QC = 512
RM = 16
RA = 32
LNR = 32
PR = 256
PW = 4
LAG = 2
GA = 5

_COPIES = ('x0', 'x1', 'xr', 'wo', 'w1a', 'w3a', 'w1b', 'w3b', 'w2')


def _ln(x):
    m = jnp.mean(x, axis=-1, keepdims=True)
    c = x - m
    v = jnp.mean(c * c, axis=-1, keepdims=True)
    return c * lax.rsqrt(v + EPS)


def _dot(a, b):
    return jnp.dot(a, b, preferred_element_type=jnp.float32)


def _aligned(i, n):
    return i * n if isinstance(i, int) else pl.multiple_of(i * n, n)


def _loop(n, fn):
    def body(i, carry):
        fn(i)
        return carry
    lax.fori_loop(0, n, body, 0)


def _spread(mxu_tasks, vpu_tasks):
    n, m = len(mxu_tasks), len(vpu_tasks)
    for i, task in enumerate(mxu_tasks):
        task()
        for v in vpu_tasks[i * m // n:(i + 1) * m // n]:
            v()


def _kernel(x_hbm, wqkv_hbm, wo_hbm, w1_hbm, w3_hbm, w2_hbm, out_hbm,
            xv, ov, wqkv, wo, w1, w3, w2, tbuf, xres, xn1, xn2, ao, qkv, hs,
            sems, osems, qsems):
    S, D = xres.shape
    F = w1.shape[-1]
    NT = D // 128
    NB = S // TM
    NU = 2 * NB
    NQ = D // PR
    NP = 3 * NQ
    Dh = D // H
    QSCALE = Dh ** -0.5 * LOG2E
    P = functools.partial

    def copy(name):
        if name in ('x0', 'x1', 'xr'):
            r = {'x0': pl.ds(0, TM), 'x1': pl.ds(TM, 2 * TM), 'xr': pl.ds(3 * TM, S - 3 * TM)}[name]
            src, dst = x_hbm.at[r], xv.at[r]
        elif name in ('wo', 'w2'):
            src, dst = (wo_hbm, wo) if name == 'wo' else (w2_hbm, w2)
        else:
            c = pl.ds(0, GA * FC) if name[2] == 'a' else pl.ds(GA * FC, F - GA * FC)
            src, dst = (w1_hbm, w1) if name[1] == '1' else (w3_hbm, w3)
            src, dst = src.at[:, c], dst.at[:, c]
        return pltpu.make_async_copy(src, dst, sems.at[_COPIES.index(name)])

    def start(*names):
        for n in names:
            copy(n).start()

    def wait(*names):
        for n in names:
            copy(n).wait()

    def piece(n):
        return n // NQ, pl.ds(_aligned(n % NQ, PR), PR)

    def qkv_copy(n):
        i, rows = piece(n)
        return pltpu.make_async_copy(
            wqkv_hbm.at[rows, pl.ds(_aligned(i, D), D)], wqkv.at[i, rows, :], qsems.at[n])

    def out_copy(b):
        rows = pl.ds(_aligned(b, TM), TM)
        return pltpu.make_async_copy(ov.at[rows], out_hbm.at[rows], osems.at[b])

    def scatter_rows(tb, v):
        for g in range(v.shape[0] // Dh):
            tb[pl.ds(g * (Dh + 1), Dh), :] = v[g * Dh:(g + 1) * Dh]

    def permute_qkv(n, tb):
        i, rows = piece(n)
        scatter_rows(tb, pltpu.bitcast(wqkv[i, rows, :], jnp.uint32).T)
        t = jnp.concatenate([tb[pl.ds(d, H, stride=Dh + 1), :] for d in range(Dh)], axis=0)
        wqkv[i, rows, :] = pltpu.bitcast(t.T, jnp.bfloat16)

    def permute_wo(j, tb):
        cols = pl.ds(_aligned(j, 128), 128)
        scatter_rows(tb, pltpu.bitcast(wo[:, cols], jnp.uint32))
        out = []
        for e in range(Dh // 2):
            a = tb[pl.ds(e, H // 2, stride=Dh + 1), :]
            b = tb[pl.ds(Dh // 2 + e, H // 2, stride=Dh + 1), :]
            out.append((a & 0xFFFF) | (b << 16))
            out.append((a >> 16) | ((b >> 16) << 16))
        wo[:, cols] = pltpu.bitcast(jnp.concatenate(out, axis=0), jnp.bfloat16)

    def rows_of(u):
        return _aligned(u % NB, TM)

    def x_in(u, r0, n, cols=slice(None)):
        rows = pl.ds(rows_of(u) + r0, n)
        return jnp.where(u < NB, xv[rows, cols].astype(jnp.float32), xres[rows, cols])

    def ln1(u, r0):
        xn1[pl.ds(r0, LNR), :] = _ln(x_in(u, r0, LNR)).astype(jnp.bfloat16)

    def ln1_first(u, r0):
        x = xv[pl.ds(u * TM + r0, LNR), :].astype(jnp.float32)
        xn1[pl.ds(r0, LNR), :] = _ln(x).astype(jnp.bfloat16)

    def ln2(u, r0):
        xn2[pl.ds(r0, LNR), :] = _ln(xres[pl.ds(rows_of(u) + r0, LNR), :]).astype(jnp.bfloat16)

    def proj(u, i, c):
        y = _dot(xn1[...], wqkv[i, :, pl.ds(c * QC, QC)])
        if i == 0:
            y = y * QSCALE
        for jj in range(QC // 128):
            j = i * NT + c * (QC // 128) + jj
            yj = y[:, jj * 128:(jj + 1) * 128]
            if i > 0:
                row0 = jnp.broadcast_to(yj[0:1, :], (HALO, 128))
                qkv[j, pl.ds(0, HALO), :] = jnp.where(u % NB == 0, row0, qkv[j, pl.ds(TM, HALO), :])
            qkv[j, pl.ds(HALO, TM), :] = yj

    def attn(u, r0, n):
        def taps(j):
            out = [None] * W
            for shift in range(0, 8, DIL):
                base = qkv[j, pl.ds(r0 + (HALO - 8 - shift), n + 8), :]
                out[shift // DIL] = base[8:]
                out[(shift + 8) // DIL] = base[:n]
            return out

        lg = [None] * W
        for j in range(NT):
            q = qkv[j, pl.ds(r0 + HALO, n), :]
            for w, k in enumerate(taps(NT + j)):
                lg[w] = q * k if j == 0 else lg[w] + q * k
        for w in range(W):
            a = lg[w]
            a = a + pltpu.roll(a, 2 * H, 1)
            a = a + pltpu.roll(a, H, 1)
            if w > 0 and (not isinstance(r0, int) or r0 < DIL * w):
                pos = rows_of(u) + r0 + lax.broadcasted_iota(jnp.int32, (n, 128), 0)
                a = jnp.where(pos >= DIL * w, a, NEG)
            lg[w] = a
        m = functools.reduce(jnp.maximum, lg)
        e = [jnp.exp2(a - m) for a in lg]
        inv = 1.0 / functools.reduce(jnp.add, e)
        p = [a * inv for a in e]
        for j in range(NT):
            o = functools.reduce(jnp.add, [pw * v for pw, v in zip(p, taps(2 * NT + j))])
            ao[pl.ds(r0, n), j * 128:(j + 1) * 128] = o.astype(jnp.bfloat16)

    def oproj(u, c, n):
        cols = pl.ds(_aligned(c, n), n)
        xres[pl.ds(rows_of(u), TM), cols] = x_in(u, 0, TM, cols) + _dot(ao[...], wo[:, cols])

    def gate_up(c):
        cols = pl.ds(c * FC, FC)
        a = xn2[...]
        hg = 0.5 * _dot(a, w1[:, cols])
        up = _dot(a, w3[:, cols])
        hs[:, cols] = (hg * (jnp.tanh(hg) + 1.0) * up).astype(jnp.bfloat16)

    def down(u, c):
        rows, cols = pl.ds(rows_of(u), TM), pl.ds(c * DC, DC)
        y = xres[rows, cols] + _dot(hs[...], w2[:, cols])
        xres[rows, cols] = y
        ov[rows, cols] = y.astype(ov.dtype)

    for n in range(PW):
        qkv_copy(n).start()
    start('x0')

    def next_piece(n):
        qkv_copy(n).wait()
        pl.when(n + PW < NP)(lambda: qkv_copy(n + PW).start())
        pl.when(n + PW == NP)(lambda: start('wo', 'x1', 'w1a', 'w3a'))

    def proj_piece(n):
        i, rows = piece(n)
        y = _dot(xn1[:, rows], wqkv[i, rows, :]) * jnp.where(i == 0, QSCALE, 1.0)
        for jj in range(NT):
            j = i * NT + jj
            yj = y[:, jj * 128:(jj + 1) * 128]
            yj = yj + jnp.where(n % NQ == 0, 0.0, qkv[j, pl.ds(HALO, TM), :])
            qkv[j, pl.ds(0, HALO), :] = jnp.broadcast_to(yj[0:1, :], (HALO, 128))
            qkv[j, pl.ds(HALO, TM), :] = yj

    def prepare(n):
        next_piece(n)
        pl.when(n == 0)(lambda: wait('x0'))
        permute_qkv(n, tbuf.at[0])
        per = TM // LNR // LAG
        for k in range(per):
            ln1_first(0, _aligned(n * per + k, LNR))
    _loop(LAG, prepare)

    def project(n):
        next_piece(n + LAG)
        proj_piece(n)
        permute_qkv(n + LAG, tbuf.at[0])
    _loop(NP - LAG, project)
    wait('wo', 'x1')
    start('w1b', 'w3b')

    def project_last(n):
        proj_piece(NP - LAG + n)
        for k in range(NT // LAG):
            permute_wo(n * (NT // LAG) + k, tbuf.at[k])
    _loop(LAG, project_last)

    def attend_first(it):
        attn(0, _aligned(it, RA), RA)
        for k in range(RA // LNR):
            ln1_first(1, _aligned(it * (RA // LNR) + k, LNR))
    _loop(TM // RA, attend_first)
    start('w2')

    def period(t, carry):
        norm2 = [P(ln2, t - 1, r0) for r0 in range(0, TM, LNR)]

        @pl.when(t < NU)
        def _():
            for c in range(D // QC):
                oproj(t - 1, c, QC)
            _spread([P(proj, t, i, c) for i in range(3) for c in range(D // QC)], norm2)

        @pl.when(t == NU)
        def _():
            _loop(D // 256, lambda c: oproj(t - 1, c, 256))
            for task in norm2:
                task()

        @pl.when(t == 1)
        def _():
            wait('w1a', 'w3a')

        _spread([P(gate_up, c) for c in range(GA)],
                [P(ln1, t + 1, r0) for r0 in range(0, TM, LNR)]
                + [P(attn, t, r0, RM) for r0 in range(0, TM, RM)])

        @pl.when(t == 1)
        def _():
            wait('w1b', 'w3b', 'w2')
            start('xr')

        for c in range(GA, F // FC):
            gate_up(c)
        for c in range(D // DC):
            down(t - 1, c)
        pl.when(t == 1)(lambda: wait('xr'))
        pl.when(t > NB)(lambda: out_copy(t - 1 - NB).start())
        return carry

    lax.fori_loop(1, NU + 1, period, 0)
    for b in range(NB):
        out_copy(b).wait()


@jax.jit
def pallas_interleave_layers__sliding_local_dilated__glu_gated_swiglu__prompt_kernel(
    A_x: jax.Array,
    A_wqkv: jax.Array,
    A_wo: jax.Array,
    B_x: jax.Array,
    B_w1: jax.Array,
    B_w3: jax.Array,
    B_w2: jax.Array,
):
    del B_x
    B, S, D = A_x.shape
    F = B_w1.shape[1]
    assert B == 1 and D == 32 * H and S % TM == 0 and S > 3 * TM and F % FC == 0 and F > GA * FC
    bf16, f32 = jnp.bfloat16, jnp.float32
    hbm = pl.BlockSpec(memory_space=pl.ANY)
    out = pl.pallas_call(
        _kernel,
        in_specs=[hbm] * 6,
        out_specs=hbm,
        out_shape=jax.ShapeDtypeStruct((S, D), A_x.dtype),
        scratch_shapes=[
            pltpu.VMEM((S, D), bf16),
            pltpu.VMEM((S, D), bf16),
            pltpu.VMEM((3, D, D), bf16),
            pltpu.VMEM((D, D), bf16),
            pltpu.VMEM((D, F), bf16),
            pltpu.VMEM((D, F), bf16),
            pltpu.VMEM((F, D), bf16),
            pltpu.VMEM((D // 128 // LAG, D + H, 128), jnp.uint32),
            pltpu.VMEM((S, D), f32),
            pltpu.VMEM((TM, D), bf16),
            pltpu.VMEM((TM, D), bf16),
            pltpu.VMEM((TM, D), bf16),
            pltpu.VMEM((3 * D // 128, HALO + TM, 128), f32),
            pltpu.VMEM((TM, F), bf16),
            pltpu.SemaphoreType.DMA((len(_COPIES),)),
            pltpu.SemaphoreType.DMA((S // TM,)),
            pltpu.SemaphoreType.DMA((3 * D // PR,)),
        ],
        compiler_params=pltpu.CompilerParams(
            vmem_limit_bytes=100 * 1024 * 1024,
            flags={"XLA_TPU_EVENLY_DISTRIBUTE_CRITICAL_NODES": True},
        ),
    )(A_x.reshape(S, D), A_wqkv, A_wo, B_w1, B_w3, B_w2)
    return out.reshape(B, S, D)
```

```python
import functools

import jax
import jax.numpy as jnp
from jax import lax
import jax.experimental.pallas as pl
import jax.experimental.pallas.tpu as pltpu

H, W, DIL = 32, 8, 2
EPS = 1e-5
LOG2E = 1.4426950408889634
NEG = -1e9 * LOG2E
HALO = 16

TM = 256
FC = 512
DC = 256
QC = 512
RM = 16
RA = 32
LNR = 32
PR = 256
PW = 4
LAG = 2
GA = 5

_COPIES = ('x0', 'x1', 'xr', 'wo', 'w1a', 'w3a', 'w1b', 'w3b', 'w2')


def _ln(x):
    m = jnp.mean(x, axis=-1, keepdims=True)
    c = x - m
    v = jnp.mean(c * c, axis=-1, keepdims=True)
    return c * lax.rsqrt(v + EPS)


def _dot(a, b):
    return jnp.dot(a, b, preferred_element_type=jnp.float32)


def _aligned(i, n):
    return i * n if isinstance(i, int) else pl.multiple_of(i * n, n)


def _loop(n, fn):
    def body(i, carry):
        fn(i)
        return carry
    lax.fori_loop(0, n, body, 0)


def _spread(mxu_tasks, vpu_tasks):
    n, m = len(mxu_tasks), len(vpu_tasks)
    for i, task in enumerate(mxu_tasks):
        task()
        for v in vpu_tasks[i * m // n:(i + 1) * m // n]:
            v()


def _kernel(x_hbm, wqkv_hbm, wo_hbm, w1_hbm, w3_hbm, w2_hbm, out_hbm,
            xv, ov, wqkv, wo, w1, w3, w2, tbuf, xres, xn1, xn2, ao, qkv, hs,
            sems, osems, qsems):
    S, D = xres.shape
    F = w1.shape[-1]
    NT = D // 128
    NB = S // TM
    NU = 2 * NB
    NQ = D // PR
    NP = 3 * NQ
    Dh = D // H
    QSCALE = Dh ** -0.5 * LOG2E
    P = functools.partial

    def copy(name):
        if name in ('x0', 'x1', 'xr'):
            r = {'x0': pl.ds(0, TM), 'x1': pl.ds(TM, 2 * TM), 'xr': pl.ds(3 * TM, S - 3 * TM)}[name]
            src, dst = x_hbm.at[r], xv.at[r]
        elif name in ('wo', 'w2'):
            src, dst = (wo_hbm, wo) if name == 'wo' else (w2_hbm, w2)
        else:
            c = pl.ds(0, GA * FC) if name[2] == 'a' else pl.ds(GA * FC, F - GA * FC)
            src, dst = (w1_hbm, w1) if name[1] == '1' else (w3_hbm, w3)
            src, dst = src.at[:, c], dst.at[:, c]
        return pltpu.make_async_copy(src, dst, sems.at[_COPIES.index(name)])

    def start(*names):
        for n in names:
            copy(n).start()

    def wait(*names):
        for n in names:
            copy(n).wait()

    def piece(n):
        return n // NQ, pl.ds(_aligned(n % NQ, PR), PR)

    def qkv_copy(n):
        i, rows = piece(n)
        return pltpu.make_async_copy(
            wqkv_hbm.at[rows, pl.ds(_aligned(i, D), D)], wqkv.at[i, rows, :], qsems.at[n])

    def out_copy(b):
        rows = pl.ds(_aligned(b, TM), TM)
        return pltpu.make_async_copy(ov.at[rows], out_hbm.at[rows], osems.at[b])

    def scatter_rows(tb, v):
        for g in range(v.shape[0] // Dh):
            tb[pl.ds(g * (Dh + 1), Dh), :] = v[g * Dh:(g + 1) * Dh]

    def permute_qkv(n, tb):
        i, rows = piece(n)
        scatter_rows(tb, pltpu.bitcast(wqkv[i, rows, :], jnp.uint32).T)
        t = jnp.concatenate([tb[pl.ds(d, H, stride=Dh + 1), :] for d in range(Dh)], axis=0)
        wqkv[i, rows, :] = pltpu.bitcast(t.T, jnp.bfloat16)

    def permute_wo(j, tb):
        cols = pl.ds(_aligned(j, 128), 128)
        scatter_rows(tb, pltpu.bitcast(wo[:, cols], jnp.uint32))
        out = []
        for e in range(Dh // 2):
            a = tb[pl.ds(e, H // 2, stride=Dh + 1), :]
            b = tb[pl.ds(Dh // 2 + e, H // 2, stride=Dh + 1), :]
            out.append((a & 0xFFFF) | (b << 16))
            out.append((a >> 16) | ((b >> 16) << 16))
        wo[:, cols] = pltpu.bitcast(jnp.concatenate(out, axis=0), jnp.bfloat16)

    def rows_of(u):
        return _aligned(u % NB, TM)

    def x_in(u, r0, n, cols=slice(None)):
        rows = pl.ds(rows_of(u) + r0, n)
        return jnp.where(u < NB, xv[rows, cols].astype(jnp.float32), xres[rows, cols])

    def ln1(u, r0):
        xn1[pl.ds(r0, LNR), :] = _ln(x_in(u, r0, LNR)).astype(jnp.bfloat16)

    def ln1_first(u, r0):
        x = xv[pl.ds(u * TM + r0, LNR), :].astype(jnp.float32)
        xn1[pl.ds(r0, LNR), :] = _ln(x).astype(jnp.bfloat16)

    def ln2(u, r0):
        xn2[pl.ds(r0, LNR), :] = _ln(xres[pl.ds(rows_of(u) + r0, LNR), :]).astype(jnp.bfloat16)

    def proj(u, i, c):
        y = _dot(xn1[...], wqkv[i, :, pl.ds(c * QC, QC)])
        if i == 0:
            y = y * QSCALE
        for jj in range(QC // 128):
            j = i * NT + c * (QC // 128) + jj
            yj = y[:, jj * 128:(jj + 1) * 128]
            if i > 0:
                row0 = jnp.broadcast_to(yj[0:1, :], (HALO, 128))
                qkv[j, pl.ds(0, HALO), :] = jnp.where(u % NB == 0, row0, qkv[j, pl.ds(TM, HALO), :])
            qkv[j, pl.ds(HALO, TM), :] = yj

    def attn(u, r0, n):
        def taps(j):
            out = [None] * W
            for shift in range(0, 8, DIL):
                base = qkv[j, pl.ds(r0 + (HALO - 8 - shift), n + 8), :]
                out[shift // DIL] = base[8:]
                out[(shift + 8) // DIL] = base[:n]
            return out

        lg = [None] * W
        for j in range(NT):
            q = qkv[j, pl.ds(r0 + HALO, n), :]
            for w, k in enumerate(taps(NT + j)):
                lg[w] = q * k if j == 0 else lg[w] + q * k
        for w in range(W):
            a = lg[w]
            a = a + pltpu.roll(a, 2 * H, 1)
            a = a + pltpu.roll(a, H, 1)
            if w > 0 and (not isinstance(r0, int) or r0 < DIL * w):
                pos = rows_of(u) + r0 + lax.broadcasted_iota(jnp.int32, (n, 128), 0)
                a = jnp.where(pos >= DIL * w, a, NEG)
            lg[w] = a
        m = functools.reduce(jnp.maximum, lg)
        e = [jnp.exp2(a - m) for a in lg]
        inv = 1.0 / functools.reduce(jnp.add, e)
        p = [a * inv for a in e]
        for j in range(NT):
            o = functools.reduce(jnp.add, [pw * v for pw, v in zip(p, taps(2 * NT + j))])
            ao[pl.ds(r0, n), j * 128:(j + 1) * 128] = o.astype(jnp.bfloat16)

    def oproj(u, c, n):
        cols = pl.ds(_aligned(c, n), n)
        xres[pl.ds(rows_of(u), TM), cols] = x_in(u, 0, TM, cols) + _dot(ao[...], wo[:, cols])

    def gate_up(c):
        cols = pl.ds(c * FC, FC)
        a = xn2[...]
        hg = 0.5 * _dot(a, w1[:, cols])
        up = _dot(a, w3[:, cols])
        hs[:, cols] = (hg * (jnp.tanh(hg) + 1.0) * up).astype(jnp.bfloat16)

    def down(u, c):
        rows, cols = pl.ds(rows_of(u), TM), pl.ds(c * DC, DC)
        y = xres[rows, cols] + _dot(hs[...], w2[:, cols])
        xres[rows, cols] = y
        ov[rows, cols] = y.astype(ov.dtype)

    qkv_copy(0).start()
    start('x0')
    qkv_copy(1).start()

    def next_piece(n):
        qkv_copy(n).wait()
        pl.when(n + PW < NP)(lambda: qkv_copy(n + PW).start())
        pl.when(n + PW == NP)(lambda: start('wo', 'x1', 'w1a', 'w3a'))

    def proj_piece(n):
        i, rows = piece(n)
        y = _dot(xn1[:, rows], wqkv[i, rows, :]) * jnp.where(i == 0, QSCALE, 1.0)
        for jj in range(NT):
            j = i * NT + jj
            yj = y[:, jj * 128:(jj + 1) * 128]
            yj = yj + jnp.where(n % NQ == 0, 0.0, qkv[j, pl.ds(HALO, TM), :])
            qkv[j, pl.ds(0, HALO), :] = jnp.broadcast_to(yj[0:1, :], (HALO, 128))
            qkv[j, pl.ds(HALO, TM), :] = yj

    def prepare(n):
        qkv_copy(n).wait()
        qkv_copy(2 * n + 2).start()
        qkv_copy(2 * n + 3).start()
        pl.when(n == 0)(lambda: wait('x0'))
        permute_qkv(n, tbuf.at[0])
        per = TM // LNR // LAG
        for k in range(per):
            ln1_first(0, _aligned(n * per + k, LNR))
    _loop(LAG, prepare)

    def project(n):
        next_piece(n + LAG)
        proj_piece(n)
        permute_qkv(n + LAG, tbuf.at[0])
    _loop(NP - LAG, project)
    wait('wo', 'x1')
    start('w1b', 'w3b')

    def project_last(n):
        proj_piece(NP - LAG + n)
        for k in range(NT // LAG):
            permute_wo(n * (NT // LAG) + k, tbuf.at[k])
    _loop(LAG, project_last)

    def attend_first(it):
        attn(0, _aligned(it, RA), RA)
        for k in range(RA // LNR):
            ln1_first(1, _aligned(it * (RA // LNR) + k, LNR))
    _loop(TM // RA, attend_first)
    start('w2')

    def period(t, carry):
        norm2 = [P(ln2, t - 1, r0) for r0 in range(0, TM, LNR)]

        @pl.when(t < NU)
        def _():
            for c in range(D // QC):
                oproj(t - 1, c, QC)
            _spread([P(proj, t, i, c) for i in range(3) for c in range(D // QC)], norm2)

        @pl.when(t == NU)
        def _():
            _loop(D // 256, lambda c: oproj(t - 1, c, 256))
            for task in norm2:
                task()

        @pl.when(t == 1)
        def _():
            wait('w1a', 'w3a')

        _spread([P(gate_up, c) for c in range(GA)],
                [P(ln1, t + 1, r0) for r0 in range(0, TM, LNR)]
                + [P(attn, t, r0, RM) for r0 in range(0, TM, RM)])

        @pl.when(t == 1)
        def _():
            wait('w1b', 'w3b', 'w2')
            start('xr')

        for c in range(GA, F // FC):
            gate_up(c)
        for c in range(D // DC):
            down(t - 1, c)
        pl.when(t == 1)(lambda: wait('xr'))
        pl.when(t > NB)(lambda: out_copy(t - 1 - NB).start())
        return carry

    lax.fori_loop(1, NU + 1, period, 0)
    for b in range(NB):
        out_copy(b).wait()


@jax.jit
def pallas_interleave_layers__sliding_local_dilated__glu_gated_swiglu__prompt_kernel(
    A_x: jax.Array,
    A_wqkv: jax.Array,
    A_wo: jax.Array,
    B_x: jax.Array,
    B_w1: jax.Array,
    B_w3: jax.Array,
    B_w2: jax.Array,
):
    del B_x
    B, S, D = A_x.shape
    F = B_w1.shape[1]
    assert B == 1 and D == 32 * H and S % TM == 0 and S > 3 * TM and F % FC == 0 and F > GA * FC
    bf16, f32 = jnp.bfloat16, jnp.float32
    hbm = pl.BlockSpec(memory_space=pl.ANY)
    out = pl.pallas_call(
        _kernel,
        in_specs=[hbm] * 6,
        out_specs=hbm,
        out_shape=jax.ShapeDtypeStruct((S, D), A_x.dtype),
        scratch_shapes=[
            pltpu.VMEM((S, D), bf16),
            pltpu.VMEM((S, D), bf16),
            pltpu.VMEM((3, D, D), bf16),
            pltpu.VMEM((D, D), bf16),
            pltpu.VMEM((D, F), bf16),
            pltpu.VMEM((D, F), bf16),
            pltpu.VMEM((F, D), bf16),
            pltpu.VMEM((D // 128 // LAG, D + 2 * H, 128), jnp.uint32),
            pltpu.VMEM((S, D), f32),
            pltpu.VMEM((TM, D), bf16),
            pltpu.VMEM((TM, D), bf16),
            pltpu.VMEM((TM, D), bf16),
            pltpu.VMEM((3 * D // 128, HALO + TM, 128), f32),
            pltpu.VMEM((TM, F), bf16),
            pltpu.SemaphoreType.DMA((len(_COPIES),)),
            pltpu.SemaphoreType.DMA((S // TM,)),
            pltpu.SemaphoreType.DMA((3 * D // PR,)),
        ],
        compiler_params=pltpu.CompilerParams(
            vmem_limit_bytes=100 * 1024 * 1024,
            flags={"XLA_TPU_EVENLY_DISTRIBUTE_CRITICAL_NODES": True},
        ),
    )(A_x.reshape(S, D), A_wqkv, A_wo, B_w1, B_w3, B_w2)
    return out.reshape(B, S, D)
```

```python
import functools

import jax
import jax.numpy as jnp
from jax import lax
import jax.experimental.pallas as pl
import jax.experimental.pallas.tpu as pltpu

H, W, DIL = 32, 8, 2
EPS = 1e-5
LOG2E = 1.4426950408889634
NEG = -1e9 * LOG2E
HALO = 16

TM = 256
FC = 512
DC = 256
QC = 512
RM = 16
RA = 32
LNR = 32
PR = 256
PW = 4
LAG = 2

_COPIES = ('x0', 'x1', 'xr', 'wo', 'w1', 'w3', 'w2')


def _ln(x):
    m = jnp.mean(x, axis=-1, keepdims=True)
    c = x - m
    v = jnp.mean(c * c, axis=-1, keepdims=True)
    return c * lax.rsqrt(v + EPS)


def _dot(a, b):
    return jnp.dot(a, b, preferred_element_type=jnp.float32)


def _aligned(i, n):
    return i * n if isinstance(i, int) else pl.multiple_of(i * n, n)


def _loop(n, fn):
    def body(i, carry):
        fn(i)
        return carry
    lax.fori_loop(0, n, body, 0)


def _spread(mxu_tasks, vpu_tasks):
    n, m = len(mxu_tasks), len(vpu_tasks)
    for i, task in enumerate(mxu_tasks):
        task()
        for v in vpu_tasks[i * m // n:(i + 1) * m // n]:
            v()


def _kernel(x_hbm, wqkv_hbm, wo_hbm, w1_hbm, w3_hbm, w2_hbm, out_hbm,
            xv, ov, wqkv, wo, w1, w3, w2, tbuf, xres, xn1, xn2, ao, qkv, hs,
            sems, osems, qsems):
    S, D = xres.shape
    F = w1.shape[-1]
    NT = D // 128
    NB = S // TM
    NU = 2 * NB
    NQ = D // PR
    NP = 3 * NQ
    Dh = D // H
    QSCALE = Dh ** -0.5 * LOG2E
    P = functools.partial

    def copy(name):
        if name in ('x0', 'x1', 'xr'):
            r = {'x0': pl.ds(0, TM), 'x1': pl.ds(TM, 2 * TM), 'xr': pl.ds(3 * TM, S - 3 * TM)}[name]
            src, dst = x_hbm.at[r], xv.at[r]
        else:
            src, dst = {'wo': (wo_hbm, wo), 'w1': (w1_hbm, w1),
                        'w3': (w3_hbm, w3), 'w2': (w2_hbm, w2)}[name]
        return pltpu.make_async_copy(src, dst, sems.at[_COPIES.index(name)])

    def start(*names):
        for n in names:
            copy(n).start()

    def wait(*names):
        for n in names:
            copy(n).wait()

    def piece(n):
        return n // NQ, pl.ds(_aligned(n % NQ, PR), PR)

    def qkv_copy(n):
        i, rows = piece(n)
        return pltpu.make_async_copy(
            wqkv_hbm.at[rows, pl.ds(_aligned(i, D), D)], wqkv.at[i, rows, :], qsems.at[n])

    def out_copy(b):
        rows = pl.ds(_aligned(b, TM), TM)
        return pltpu.make_async_copy(ov.at[rows], out_hbm.at[rows], osems.at[b])

    def scatter_rows(tb, v):
        for g in range(v.shape[0] // Dh):
            tb[pl.ds(g * (Dh + 1), Dh), :] = v[g * Dh:(g + 1) * Dh]

    def permute_qkv(n, tb):
        i, rows = piece(n)
        scatter_rows(tb, pltpu.bitcast(wqkv[i, rows, :], jnp.uint32).T)
        t = jnp.concatenate([tb[pl.ds(d, H, stride=Dh + 1), :] for d in range(Dh)], axis=0)
        wqkv[i, rows, :] = pltpu.bitcast(t.T, jnp.bfloat16)

    def permute_wo(j, tb):
        cols = pl.ds(_aligned(j, 128), 128)
        scatter_rows(tb, pltpu.bitcast(wo[:, cols], jnp.uint32))
        out = []
        for e in range(Dh // 2):
            a = tb[pl.ds(e, H // 2, stride=Dh + 1), :]
            b = tb[pl.ds(Dh // 2 + e, H // 2, stride=Dh + 1), :]
            out.append((a & 0xFFFF) | (b << 16))
            out.append((a >> 16) | ((b >> 16) << 16))
        wo[:, cols] = pltpu.bitcast(jnp.concatenate(out, axis=0), jnp.bfloat16)

    def rows_of(u):
        return _aligned(u % NB, TM)

    def x_in(u, r0, n, cols=slice(None)):
        rows = pl.ds(rows_of(u) + r0, n)
        return jnp.where(u < NB, xv[rows, cols].astype(jnp.float32), xres[rows, cols])

    def ln1(u, r0):
        xn1[pl.ds(r0, LNR), :] = _ln(x_in(u, r0, LNR)).astype(jnp.bfloat16)

    def ln1_first(u, r0):
        x = xv[pl.ds(_aligned(u, TM) + r0, LNR), :].astype(jnp.float32)
        xn1[pl.ds(r0, LNR), :] = _ln(x).astype(jnp.bfloat16)

    def ln2(u, r0):
        xn2[pl.ds(r0, LNR), :] = _ln(xres[pl.ds(rows_of(u) + r0, LNR), :]).astype(jnp.bfloat16)

    def proj(u, i, c):
        y = _dot(xn1[...], wqkv[i, :, pl.ds(c * QC, QC)])
        if i == 0:
            y = y * QSCALE
        for jj in range(QC // 128):
            j = i * NT + c * (QC // 128) + jj
            yj = y[:, jj * 128:(jj + 1) * 128]
            if i > 0:
                row0 = jnp.broadcast_to(yj[0:1, :], (HALO, 128))
                qkv[j, pl.ds(0, HALO), :] = jnp.where(u % NB == 0, row0, qkv[j, pl.ds(TM, HALO), :])
            qkv[j, pl.ds(HALO, TM), :] = yj

    def attn(u, r0, n):
        def taps(j):
            out = [None] * W
            for shift in range(0, 8, DIL):
                base = qkv[j, pl.ds(r0 + (HALO - 8 - shift), n + 8), :]
                out[shift // DIL] = base[8:]
                out[(shift + 8) // DIL] = base[:n]
            return out

        lg = [None] * W
        for j in range(NT):
            q = qkv[j, pl.ds(r0 + HALO, n), :]
            for w, k in enumerate(taps(NT + j)):
                lg[w] = q * k if j == 0 else lg[w] + q * k
        for w in range(W):
            a = lg[w]
            a = a + pltpu.roll(a, 2 * H, 1)
            a = a + pltpu.roll(a, H, 1)
            if w > 0 and (not isinstance(r0, int) or r0 < DIL * w):
                pos = rows_of(u) + r0 + lax.broadcasted_iota(jnp.int32, (n, 128), 0)
                a = jnp.where(pos >= DIL * w, a, NEG)
            lg[w] = a
        m = functools.reduce(jnp.maximum, lg)
        e = [jnp.exp2(a - m) for a in lg]
        inv = 1.0 / functools.reduce(jnp.add, e)
        p = [a * inv for a in e]
        for j in range(NT):
            o = functools.reduce(jnp.add, [pw * v for pw, v in zip(p, taps(2 * NT + j))])
            ao[pl.ds(r0, n), j * 128:(j + 1) * 128] = o.astype(jnp.bfloat16)

    def oproj(u, c, n):
        cols = pl.ds(_aligned(c, n), n)
        xres[pl.ds(rows_of(u), TM), cols] = x_in(u, 0, TM, cols) + _dot(ao[...], wo[:, cols])

    def gate_up(c):
        cols = pl.ds(c * FC, FC)
        a = xn2[...]
        hg = 0.5 * _dot(a, w1[:, cols])
        up = _dot(a, w3[:, cols])
        hs[:, cols] = (hg * (jnp.tanh(hg) + 1.0) * up).astype(jnp.bfloat16)

    def down(u, c):
        rows, cols = pl.ds(rows_of(u), TM), pl.ds(c * DC, DC)
        y = xres[rows, cols] + _dot(hs[...], w2[:, cols])
        xres[rows, cols] = y
        ov[rows, cols] = y.astype(ov.dtype)

    qkv_copy(0).start()
    start('x0')
    qkv_copy(1).start()
    xres[pl.ds(0, TM), :] = jnp.zeros((TM, D), jnp.float32)

    def next_piece(n):
        qkv_copy(n).wait()
        pl.when(n + PW < NP)(lambda: qkv_copy(n + PW).start())
        pl.when(n + PW == NP)(lambda: start('wo', 'x1', 'w1'))

    def proj_piece(n):
        i, rows = piece(n)
        y = _dot(xn1[:, rows], wqkv[i, rows, :]) * jnp.where(i == 0, QSCALE, 1.0)
        for jj in range(NT):
            j = i * NT + jj
            yj = y[:, jj * 128:(jj + 1) * 128]
            yj = yj + jnp.where(n % NQ == 0, 0.0, qkv[j, pl.ds(HALO, TM), :])
            qkv[j, pl.ds(0, HALO), :] = jnp.broadcast_to(yj[0:1, :], (HALO, 128))
            qkv[j, pl.ds(HALO, TM), :] = yj

    def prepare(n):
        qkv_copy(n).wait()
        qkv_copy(2 * n + 2).start()
        qkv_copy(2 * n + 3).start()
        pl.when(n == 0)(lambda: wait('x0'))
        permute_qkv(n, tbuf.at[0])
        per = TM // LNR // LAG
        for k in range(per):
            ln1_first(0, _aligned(n * per + k, LNR))
    _loop(LAG, prepare)

    def project(n):
        next_piece(n + LAG)
        proj_piece(n)
        permute_qkv(n + LAG, tbuf.at[0])
    _loop(NP - LAG, project)
    wait('wo', 'x1')
    start('w3', 'w2', 'xr')

    def project_last(n):
        proj_piece(NP - LAG + n)
        for k in range(NT // LAG):
            permute_wo(n * (NT // LAG) + k, tbuf.at[k])
    _loop(LAG, project_last)

    def period(t, carry):
        norm2 = [P(ln2, jnp.maximum(t - 2, 0), r0) for r0 in range(0, TM, LNR)]

        @pl.when((t > 0) & (t < NU))
        def _():
            _spread([P(proj, t, i, c) for i in range(3) for c in range(D // QC)], norm2)
            for c in range(D // QC):
                oproj(t - 1, c, QC)

        @pl.when(t == NU)
        def _():
            _loop(D // 256, lambda c: oproj(t - 1, c, 256))

        @pl.when(t >= NU)
        def _():
            for task in norm2:
                task()

        @pl.when(t < 2)
        def _():
            def attend(it):
                attn(t, _aligned(it, RA), RA)
                for k in range(RA // LNR):
                    ln1_first(t + 1, _aligned(it * (RA // LNR) + k, LNR))
            _loop(TM // RA, attend)

        pl.when(t == 2)(lambda: wait('w1', 'w3', 'w2', 'xr'))

        @pl.when(t >= 2)
        def _():
            _spread([P(gate_up, c) for c in range(F // FC)],
                    [P(ln1, t + 1, r0) for r0 in range(0, TM, LNR)]
                    + [P(attn, t, r0, RM) for r0 in range(0, TM, RM)])
            for c in range(D // DC):
                down(t - 2, c)

        pl.when(t >= NB + 2)(lambda: out_copy(t - 2 - NB).start())
        return carry

    lax.fori_loop(0, NU + 2, period, 0)
    for b in range(NB):
        out_copy(b).wait()


@jax.jit
def pallas_interleave_layers__sliding_local_dilated__glu_gated_swiglu__prompt_kernel(
    A_x: jax.Array,
    A_wqkv: jax.Array,
    A_wo: jax.Array,
    B_x: jax.Array,
    B_w1: jax.Array,
    B_w3: jax.Array,
    B_w2: jax.Array,
):
    del B_x
    B, S, D = A_x.shape
    F = B_w1.shape[1]
    assert B == 1 and D == 32 * H and S % TM == 0 and S > 3 * TM and F % FC == 0
    bf16, f32 = jnp.bfloat16, jnp.float32
    hbm = pl.BlockSpec(memory_space=pl.ANY)
    out = pl.pallas_call(
        _kernel,
        in_specs=[hbm] * 6,
        out_specs=hbm,
        out_shape=jax.ShapeDtypeStruct((S, D), A_x.dtype),
        scratch_shapes=[
            pltpu.VMEM((S, D), bf16),
            pltpu.VMEM((S, D), bf16),
            pltpu.VMEM((3, D, D), bf16),
            pltpu.VMEM((D, D), bf16),
            pltpu.VMEM((D, F), bf16),
            pltpu.VMEM((D, F), bf16),
            pltpu.VMEM((F, D), bf16),
            pltpu.VMEM((D // 128 // LAG, D + 2 * H, 128), jnp.uint32),
            pltpu.VMEM((S, D), f32),
            pltpu.VMEM((TM, D), bf16),
            pltpu.VMEM((TM, D), bf16),
            pltpu.VMEM((TM, D), bf16),
            pltpu.VMEM((3 * D // 128, HALO + TM, 128), f32),
            pltpu.VMEM((TM, F), bf16),
            pltpu.SemaphoreType.DMA((len(_COPIES),)),
            pltpu.SemaphoreType.DMA((S // TM,)),
            pltpu.SemaphoreType.DMA((3 * D // PR,)),
        ],
        compiler_params=pltpu.CompilerParams(
            vmem_limit_bytes=100 * 1024 * 1024,
            flags={"XLA_TPU_EVENLY_DISTRIBUTE_CRITICAL_NODES": True},
        ),
    )(A_x.reshape(S, D), A_wqkv, A_wo, B_w1, B_w3, B_w2)
    return out.reshape(B, S, D)
```

```python
import functools

import jax
import jax.numpy as jnp
from jax import lax
import jax.experimental.pallas as pl
import jax.experimental.pallas.tpu as pltpu

H, W, DIL = 32, 8, 2
EPS = 1e-5
LOG2E = 1.4426950408889634
NEG = -1e9 * LOG2E
HALO = 16

TM = 256
FC = 512
DC = 256
QC = 512
RM = 16
RA = 32
LNR = 32
PR = 256
PW = 4
LAG = 2

_COPIES = ('x0', 'x1', 'xr', 'wo', 'w1', 'w3', 'w2')


def _ln(x):
    m = jnp.mean(x, axis=-1, keepdims=True)
    c = x - m
    v = jnp.mean(c * c, axis=-1, keepdims=True)
    return c * lax.rsqrt(v + EPS)


def _dot(a, b):
    return jnp.dot(a, b, preferred_element_type=jnp.float32)


def _aligned(i, n):
    return i * n if isinstance(i, int) else pl.multiple_of(i * n, n)


def _loop(n, fn):
    def body(i, carry):
        fn(i)
        return carry
    lax.fori_loop(0, n, body, 0)


def _spread(mxu_tasks, vpu_tasks):
    n, m = len(mxu_tasks), len(vpu_tasks)
    for i, task in enumerate(mxu_tasks):
        task()
        for v in vpu_tasks[i * m // n:(i + 1) * m // n]:
            v()


def _kernel(x_hbm, wqkv_hbm, wo_hbm, w1_hbm, w3_hbm, w2_hbm, out_hbm,
            xv, ov, wqkv, wo, w1, w3, w2, tbuf, xres, xn1, xn2, ao, qkv, hs,
            sems, osems, qsems):
    S, D = xres.shape
    F = w1.shape[-1]
    NT = D // 128
    NB = S // TM
    NU = 2 * NB
    NQ = D // PR
    NP = 3 * NQ
    Dh = D // H
    QSCALE = Dh ** -0.5 * LOG2E
    P = functools.partial

    def copy(name):
        if name in ('x0', 'x1', 'xr'):
            r = {'x0': pl.ds(0, TM), 'x1': pl.ds(TM, 2 * TM), 'xr': pl.ds(3 * TM, S - 3 * TM)}[name]
            src, dst = x_hbm.at[r], xv.at[r]
        else:
            src, dst = {'wo': (wo_hbm, wo), 'w1': (w1_hbm, w1),
                        'w3': (w3_hbm, w3), 'w2': (w2_hbm, w2)}[name]
        return pltpu.make_async_copy(src, dst, sems.at[_COPIES.index(name)])

    def start(*names):
        for n in names:
            copy(n).start()

    def wait(*names):
        for n in names:
            copy(n).wait()

    def piece(n):
        return n // NQ, pl.ds(_aligned(n % NQ, PR), PR)

    def qkv_copy(n):
        i, rows = piece(n)
        return pltpu.make_async_copy(
            wqkv_hbm.at[rows, pl.ds(_aligned(i, D), D)], wqkv.at[i, rows, :], qsems.at[n])

    def out_copy(b):
        rows = pl.ds(_aligned(b, TM), TM)
        return pltpu.make_async_copy(ov.at[rows], out_hbm.at[rows], osems.at[b])

    def scatter_rows(tb, v):
        for g in range(v.shape[0] // Dh):
            tb[pl.ds(g * (Dh + 1), Dh), :] = v[g * Dh:(g + 1) * Dh]

    def permute_qkv(n, tb):
        i, rows = piece(n)
        scatter_rows(tb, pltpu.bitcast(wqkv[i, rows, :], jnp.uint32).T)
        t = jnp.concatenate([tb[pl.ds(d, H, stride=Dh + 1), :] for d in range(Dh)], axis=0)
        wqkv[i, rows, :] = pltpu.bitcast(t.T, jnp.bfloat16)

    def permute_wo(j, tb):
        cols = pl.ds(_aligned(j, 128), 128)
        scatter_rows(tb, pltpu.bitcast(wo[:, cols], jnp.uint32))
        out = []
        for e in range(Dh // 2):
            a = tb[pl.ds(e, H // 2, stride=Dh + 1), :]
            b = tb[pl.ds(Dh // 2 + e, H // 2, stride=Dh + 1), :]
            out.append((a & 0xFFFF) | (b << 16))
            out.append((a >> 16) | ((b >> 16) << 16))
        wo[:, cols] = pltpu.bitcast(jnp.concatenate(out, axis=0), jnp.bfloat16)

    def rows_of(u):
        return _aligned(u % NB, TM)

    def x_in(u, r0, n, cols=slice(None)):
        rows = pl.ds(rows_of(u) + r0, n)
        return jnp.where(u < NB, xv[rows, cols].astype(jnp.float32), xres[rows, cols])

    def ln1(u, r0):
        xn1[pl.ds(r0, LNR), :] = _ln(x_in(u, r0, LNR)).astype(jnp.bfloat16)

    def ln1_first(u, r0):
        x = xv[pl.ds(_aligned(u, TM) + r0, LNR), :].astype(jnp.float32)
        xn1[pl.ds(r0, LNR), :] = _ln(x).astype(jnp.bfloat16)

    def ln2(u, r0):
        xn2[pl.ds(r0, LNR), :] = _ln(xres[pl.ds(rows_of(u) + r0, LNR), :]).astype(jnp.bfloat16)

    def proj(u, i, c):
        y = _dot(xn1[...], wqkv[i, :, pl.ds(c * QC, QC)])
        if i == 0:
            y = y * QSCALE
        for jj in range(QC // 128):
            j = i * NT + c * (QC // 128) + jj
            yj = y[:, jj * 128:(jj + 1) * 128]
            if i > 0:
                row0 = jnp.broadcast_to(yj[0:1, :], (HALO, 128))
                qkv[j, pl.ds(0, HALO), :] = jnp.where(u % NB == 0, row0, qkv[j, pl.ds(TM, HALO), :])
            qkv[j, pl.ds(HALO, TM), :] = yj

    def attn(u, r0, n):
        def taps(j):
            out = [None] * W
            for shift in range(0, 8, DIL):
                base = qkv[j, pl.ds(r0 + (HALO - 8 - shift), n + 8), :]
                out[shift // DIL] = base[8:]
                out[(shift + 8) // DIL] = base[:n]
            return out

        lg = [None] * W
        for j in range(NT):
            q = qkv[j, pl.ds(r0 + HALO, n), :]
            for w, k in enumerate(taps(NT + j)):
                lg[w] = q * k if j == 0 else lg[w] + q * k
        for w in range(W):
            a = lg[w]
            a = a + pltpu.roll(a, 2 * H, 1)
            a = a + pltpu.roll(a, H, 1)
            if w > 0 and (not isinstance(r0, int) or r0 < DIL * w):
                pos = rows_of(u) + r0 + lax.broadcasted_iota(jnp.int32, (n, 128), 0)
                a = jnp.where(pos >= DIL * w, a, NEG)
            lg[w] = a
        m = functools.reduce(jnp.maximum, lg)
        e = [jnp.exp2(a - m) for a in lg]
        inv = 1.0 / functools.reduce(jnp.add, e)
        p = [a * inv for a in e]
        for j in range(NT):
            o = functools.reduce(jnp.add, [pw * v for pw, v in zip(p, taps(2 * NT + j))])
            ao[pl.ds(r0, n), j * 128:(j + 1) * 128] = o.astype(jnp.bfloat16)

    def oproj(u, c, n):
        cols = pl.ds(_aligned(c, n), n)
        xres[pl.ds(rows_of(u), TM), cols] = x_in(u, 0, TM, cols) + _dot(ao[...], wo[:, cols])

    def gate_up(c):
        cols = pl.ds(c * FC, FC)
        a = xn2[...]
        hg = 0.5 * _dot(a, w1[:, cols])
        up = _dot(a, w3[:, cols])
        hs[:, cols] = (hg * (jnp.tanh(hg) + 1.0) * up).astype(jnp.bfloat16)

    def down(u, c):
        rows, cols = pl.ds(rows_of(u), TM), pl.ds(c * DC, DC)
        y = xres[rows, cols] + _dot(hs[...], w2[:, cols])
        xres[rows, cols] = y
        ov[rows, cols] = y.astype(ov.dtype)

    qkv_copy(0).start()
    start('x0')
    qkv_copy(1).start()
    xres[pl.ds(0, TM), :] = jnp.zeros((TM, D), jnp.float32)

    def next_piece(n):
        qkv_copy(n).wait()
        pl.when(n + PW < NP)(lambda: qkv_copy(n + PW).start())
        pl.when(n + PW == NP)(lambda: start('wo', 'x1', 'w1'))

    def proj_piece(n):
        i, rows = piece(n)
        y = _dot(xn1[:, rows], wqkv[i, rows, :]) * jnp.where(i == 0, QSCALE, 1.0)
        for jj in range(NT):
            j = i * NT + jj
            yj = y[:, jj * 128:(jj + 1) * 128]
            yj = yj + jnp.where(n % NQ == 0, 0.0, qkv[j, pl.ds(HALO, TM), :])
            qkv[j, pl.ds(0, HALO), :] = jnp.broadcast_to(yj[0:1, :], (HALO, 128))
            qkv[j, pl.ds(HALO, TM), :] = yj

    def prepare(n):
        qkv_copy(n).wait()
        qkv_copy(2 * n + 2).start()
        qkv_copy(2 * n + 3).start()
        pl.when(n == 0)(lambda: wait('x0'))
        permute_qkv(n, tbuf.at[0])
        per = TM // LNR // LAG
        for k in range(per):
            ln1_first(0, _aligned(n * per + k, LNR))
    _loop(LAG, prepare)

    def project(n):
        next_piece(n + LAG)
        proj_piece(n)
        permute_qkv(n + LAG, tbuf.at[0])
    _loop(NP - LAG, project)
    wait('wo', 'x1')
    start('w3', 'w2', 'xr')

    def project_last(n):
        proj_piece(NP - LAG + n)
        for k in range(NT // LAG):
            permute_wo(n * (NT // LAG) + k, tbuf.at[k])
    _loop(LAG, project_last)

    def period(t, carry):
        norm2 = [P(ln2, jnp.maximum(t - 2, 0), r0) for r0 in range(0, TM, LNR)]

        @pl.when((t > 0) & (t < NU))
        def _():
            _spread([P(proj, t, i, c) for i in range(3) for c in range(D // QC)], norm2)
            for c in range(D // QC):
                oproj(t - 1, c, QC)

        @pl.when((t <= 2) | (t >= NU))
        def _():
            @pl.when(t == NU)
            def _():
                _loop(D // 256, lambda c: oproj(t - 1, c, 256))

            @pl.when(t >= NU)
            def _():
                for task in norm2:
                    task()

            @pl.when(t < 2)
            def _():
                def attend(it):
                    attn(t, _aligned(it, RA), RA)
                    for k in range(RA // LNR):
                        ln1_first(t + 1, _aligned(it * (RA // LNR) + k, LNR))
                _loop(TM // RA, attend)

            pl.when(t == 2)(lambda: wait('w1', 'w3', 'w2', 'xr'))

        @pl.when(t >= 2)
        def _():
            _spread([P(gate_up, c) for c in range(F // FC)],
                    [P(ln1, t + 1, r0) for r0 in range(0, TM, LNR)]
                    + [P(attn, t, r0, RM) for r0 in range(0, TM, RM)])
            for c in range(D // DC):
                down(t - 2, c)

        pl.when(t >= NB + 2)(lambda: out_copy(t - 2 - NB).start())
        return carry

    lax.fori_loop(0, NU + 2, period, 0)
    for b in range(NB):
        out_copy(b).wait()


@jax.jit
def pallas_interleave_layers__sliding_local_dilated__glu_gated_swiglu__prompt_kernel(
    A_x: jax.Array,
    A_wqkv: jax.Array,
    A_wo: jax.Array,
    B_x: jax.Array,
    B_w1: jax.Array,
    B_w3: jax.Array,
    B_w2: jax.Array,
):
    del B_x
    B, S, D = A_x.shape
    F = B_w1.shape[1]
    assert B == 1 and D == 32 * H and S % TM == 0 and S > 3 * TM and F % FC == 0
    bf16, f32 = jnp.bfloat16, jnp.float32
    hbm = pl.BlockSpec(memory_space=pl.ANY)
    out = pl.pallas_call(
        _kernel,
        in_specs=[hbm] * 6,
        out_specs=hbm,
        out_shape=jax.ShapeDtypeStruct((S, D), A_x.dtype),
        scratch_shapes=[
            pltpu.VMEM((S, D), bf16),
            pltpu.VMEM((S, D), bf16),
            pltpu.VMEM((3, D, D), bf16),
            pltpu.VMEM((D, D), bf16),
            pltpu.VMEM((D, F), bf16),
            pltpu.VMEM((D, F), bf16),
            pltpu.VMEM((F, D), bf16),
            pltpu.VMEM((D // 128 // LAG, D + 2 * H, 128), jnp.uint32),
            pltpu.VMEM((S, D), f32),
            pltpu.VMEM((TM, D), bf16),
            pltpu.VMEM((TM, D), bf16),
            pltpu.VMEM((TM, D), bf16),
            pltpu.VMEM((3 * D // 128, HALO + TM, 128), f32),
            pltpu.VMEM((TM, F), bf16),
            pltpu.SemaphoreType.DMA((len(_COPIES),)),
            pltpu.SemaphoreType.DMA((S // TM,)),
            pltpu.SemaphoreType.DMA((3 * D // PR,)),
        ],
        compiler_params=pltpu.CompilerParams(
            vmem_limit_bytes=100 * 1024 * 1024,
            flags={"XLA_TPU_EVENLY_DISTRIBUTE_CRITICAL_NODES": True},
        ),
    )(A_x.reshape(S, D), A_wqkv, A_wo, B_w1, B_w3, B_w2)
    return out.reshape(B, S, D)
```
